```python
import jax
import jax.numpy as jnp

def _softmax(x, axis=-1):
    return jax.nn.softmax(x, axis=axis)

def _gelu(x):
    return jax.nn.gelu(x, approximate=True)

def _silu(x):
    return jax.nn.silu(x)

def _sigmoid(x):
    return jax.nn.sigmoid(x)

def _layernorm(x, axis=-1, eps=1e-05):
    m = jnp.mean(x, axis=axis, keepdims=True)
    v = jnp.var(x, axis=axis, keepdims=True)
    return (x - m) / jnp.sqrt(v + eps)

def _scatter_add(tgt, idx, src, axis=0):
    return tgt.at[idx].add(src)

def _segment_sum(src, seg, n):
    return jax.ops.segment_sum(src, seg, n)

class _Rng:

    def __init__(self, key):
        self._k = key

    def _next(self):
        self._k, sub = jax.random.split(self._k)
        return sub

    def normal(self, shape):
        return jax.random.normal(self._next(), shape, dtype=jnp.bfloat16)

    def randint(self, lo, hi, shape):
        return jax.random.randint(self._next(), shape, lo, hi, dtype=jnp.int32)

    def uniform(self, shape, lo=0.0, hi=1.0):
        return jax.random.uniform(self._next(), shape, jnp.bfloat16, lo, hi)

    def permutation(self, n):
        return jax.random.permutation(self._next(), n)
kernel_name = 'adaLN_cond__sliding_block_cached__dense_activation_gelu__decode'

def setup_inputs():
    _rng = _Rng(jax.random.key(int.from_bytes(__import__("os").urandom(4), "little")))
    _w = lambda a: (lambda t: t.astype(jnp.bfloat16) if jnp.issubdtype(t.dtype, jnp.floating) else t)(jnp.asarray(a))

    def _A_setup():
        B, Sq, D = (4, 1, 640)
        Hq, Hkv, Sk, Dh = (32, 32, 8192, 128)
        assert Hq % Hkv == 0, (Hq, Hkv)
        return {'x': _w((lambda *s: _rng.normal(s) * 0.05)(B, Sq, D)), 'k_cache': _w((lambda *s: _rng.normal(s) * 0.05)(B, Hkv, Sk, Dh)), 'v_cache': _w((lambda *s: _rng.normal(s) * 0.05)(B, Hkv, Sk, Dh)), 'wq': _w((lambda *s: _rng.normal(s) * 0.05)(D, Hq * Dh) * D ** (-0.5)), 'wo': _w((lambda *s: _rng.normal(s) * 0.05)(Hq * Dh, D) * (Hq * Dh) ** (-0.5))}
    _A_in = _A_setup()

    def _B_setup():
        B, S, D, F = (4, 1, 640, 1728)
        return {'x': _w((lambda *s: _rng.normal(s) * 0.05)(B, S, D)), 'w1': _w((lambda *s: _rng.normal(s) * 0.05)(D, F) * D ** (-0.5)), 'b1': _w((lambda *s: _rng.normal(s) * 0.05)(F) * 0.01), 'w2': _w((lambda *s: _rng.normal(s) * 0.05)(F, D) * F ** (-0.5)), 'b2': _w((lambda *s: _rng.normal(s) * 0.05)(D) * 0.01)}
    _B_in = _B_setup()
    return {'A_x': _A_in['x'], 'A_k_cache': _A_in['k_cache'], 'A_v_cache': _A_in['v_cache'], 'A_wq': _A_in['wq'], 'A_wo': _A_in['wo'], 'B_x': _B_in['x'], 'B_w1': _B_in['w1'], 'B_b1': _B_in['b1'], 'B_w2': _B_in['w2'], 'B_b2': _B_in['b2'], 'c': _w((lambda *s: _rng.normal(s) * 0.05)(4, 640)), 'w_mod': _w((lambda *s: _rng.normal(s) * 0.05)(640, 6 * 640) * 640 ** (-0.5))}

def reference(A_x, A_k_cache, A_v_cache, A_wq, A_wo, B_x, B_w1, B_b1, B_w2, B_b2, c, w_mod):

    def _A_ref(x, k_cache, v_cache, wq, wo):
        B, Sq, D = x.shape
        Hq, Dh = (32, 128)
        Hkv, Sk = (k_cache.shape[1], k_cache.shape[2])
        W = min(4096, max(256, Sk // 4))
        rep = Hq // Hkv
        q = (lambda x, *d: x.transpose(*d))((x @ wq).reshape(B, Sq, Hq, Dh), 0, 2, 1, 3)
        k = jnp.repeat(k_cache[:, :, Sk - W:, :], rep, axis=1)
        v = jnp.repeat(v_cache[:, :, Sk - W:, :], rep, axis=1)
        scores = jnp.einsum('bhqd,bhkd->bhqk', q, k) * Dh ** (-0.5)
        p = _softmax(scores, axis=-1)
        o = jnp.einsum('bhqk,bhkd->bhqd', p, v)
        return (lambda x, *d: x.transpose(*d))(o, 0, 2, 1, 3).reshape(B, Sq, Hq * Dh) @ wo

    def _B_ref(x, w1, b1, w2, b2):
        h = jnp.einsum('bsd,df->bsf', x, w1) + b1
        h = _gelu(h)
        return jnp.einsum('bsf,fd->bsd', h, w2) + b2
    x = A_x
    mod = (_silu(c) @ w_mod).reshape(c.shape[0], 6, 1, -1)
    sa, ca, ga, sb, cb, gb = (mod[:, 0].copy(), mod[:, 1].copy(), mod[:, 2].copy(), mod[:, 3].copy(), mod[:, 4].copy(), mod[:, 5].copy())
    h = _layernorm(x, axis=-1) * (1 + ca) + sa
    x = x + ga * _A_ref(h, A_k_cache, A_v_cache, A_wq, A_wo)
    h = _layernorm(x, axis=-1) * (1 + cb) + sb
    x = x + gb * _B_ref(h, B_w1, B_b1, B_w2, B_b2)
    return x
```

```python
import functools
import jax
import jax.numpy as jnp
from jax import lax
import jax.experimental.pallas as pl
import jax.experimental.pallas.tpu as pltpu

B, D, H, S, DH, F = 4, 640, 32, 8192, 128, 1728
W = 2048
NBUF = 4
EPS = 1e-5
bf16 = jnp.bfloat16
f32 = jnp.float32


def _ln(x):
    m = jnp.mean(x, axis=-1, keepdims=True)
    xc = x - m
    v = jnp.mean(xc * xc, axis=-1, keepdims=True)
    return xc / jnp.sqrt(v + EPS)


def kernel(x_hbm, c_hbm, b1_hbm, b2_hbm, k_hbm, v_hbm, wq_hbm, wo_hbm, w1_hbm, w2_hbm, wmod_hbm,
           o_hbm,
           x_v, c_v, b1_v, b2_v, wq_v, wo_v, w1_v, w2_v, wmod_v, kbuf, vbuf, q_s, o_s, out_v, wsem, ksem, vsem):
    def cp(src, dst, i):
        return pltpu.make_async_copy(src, dst, wsem.at[i])
    small = [cp(x_hbm, x_v, 0), cp(c_hbm, c_v, 1), cp(b1_hbm, b1_v, 2), cp(b2_hbm, b2_v, 3)]
    c_wmod = cp(wmod_hbm, wmod_v, 4)
    c_wq = cp(wq_hbm, wq_v, 5)
    c_wo = cp(wo_hbm, wo_v, 6)
    c_w1 = cp(w1_hbm, w1_v, 7)
    c_w2 = cp(w2_hbm, w2_v, 8)

    def kv_copy(u, slot):
        h = u // B
        b = u % B
        j = b * H + h
        return (pltpu.make_async_copy(k_hbm.at[j, pl.ds(S - W, W), :], kbuf.at[slot], ksem.at[slot]),
                pltpu.make_async_copy(v_hbm.at[j, pl.ds(S - W, W), :], vbuf.at[slot], vsem.at[slot]))

    for s in small:
        s.start()
    c_wmod.start()
    c_wq.start()
    for u in range(NBUF):
        a, b_ = kv_copy(u, u)
        a.start(); b_.start()

    for s in small:
        s.wait()
    c_wmod.wait()
    cvec = c_v[...].astype(f32)
    sc = (cvec * jax.nn.sigmoid(cvec)).astype(bf16)
    mod = jnp.dot(sc, wmod_v[...], preferred_element_type=f32)
    sa, ca, ga, sb, cb, gb = [mod[:, i * D:(i + 1) * D] for i in range(6)]
    x = x_v[...].astype(f32)
    h1 = (_ln(x) * (1.0 + ca) + sa).astype(bf16)
    c_wq.wait()
    q = jnp.dot(h1, wq_v[...], preferred_element_type=f32)
    for h in range(H):
        q_s[h, 0:B, :] = q[:, h * DH:(h + 1) * DH]
        q_s[h, B:8, :] = jnp.zeros((8 - B, DH), f32)
    o_s[...] = jnp.zeros(o_s.shape, f32)

    scale = DH ** -0.5
    NU = B * H

    def body(u, carry):
        slot = u % NBUF
        h = u // B
        b = u % B
        ck, cv = kv_copy(u, slot)
        ck.wait()
        qh = q_s[h].astype(bf16)
        s = lax.dot_general(qh, kbuf[slot], (((1,), (1,)), ((), ())), preferred_element_type=f32)
        s = s * scale
        m = jnp.max(s, axis=-1, keepdims=True)
        p = jnp.exp(s - m)
        l = jnp.sum(p, axis=-1, keepdims=True)
        cv.wait()
        o = jnp.dot(p.astype(bf16), vbuf[slot], preferred_element_type=f32)
        o = o / l
        row = lax.broadcasted_iota(jnp.int32, (8, DH), 0)
        o_s[h] = jnp.where(row == b, o, o_s[h])

        @pl.when(u + NBUF < NU)
        def _():
            a, b_ = kv_copy(u + NBUF, slot)
            a.start(); b_.start()

        @pl.when(u + NBUF == NU)
        def _():
            c_wo.start(); c_w1.start(); c_w2.start()
        return carry

    lax.fori_loop(0, NU, body, 0)

    c_wo.wait()
    oall = jnp.concatenate([o_s[h] for h in range(H)], axis=1).astype(bf16)
    att = jnp.dot(oall, wo_v[...], preferred_element_type=f32)[0:B]
    x2 = x + ga * att
    h2 = (_ln(x2) * (1.0 + cb) + sb).astype(bf16)
    c_w1.wait()
    hh = lax.dot_general(h2, w1_v[...], (((1,), (1,)), ((), ())), preferred_element_type=f32) + b1_v[...].astype(f32).reshape(1, F)
    hh = jax.nn.gelu(hh, approximate=True).astype(bf16)
    c_w2.wait()
    y = jnp.dot(hh, w2_v[...], preferred_element_type=f32) + b2_v[...].astype(f32).reshape(1, D)
    out_v[...] = (x2 + gb * y).astype(bf16)
    co = pltpu.make_async_copy(out_v, o_hbm, wsem.at[9])
    co.start(); co.wait()


@jax.jit
def pallas_adaLN_cond__sliding_block_cached__dense_activation_gelu__decode_kernel(A_x, A_k_cache, A_v_cache, A_wq, A_wo, B_x, B_w1, B_b1, B_w2, B_b2, c, w_mod):
    k = A_k_cache.reshape(B * H, S, DH)
    v = A_v_cache.reshape(B * H, S, DH)
    x = A_x.reshape(B, D)
    out = pl.pallas_call(
        kernel,
        in_specs=[pl.BlockSpec(memory_space=pl.ANY)] * 11,
        out_specs=pl.BlockSpec(memory_space=pl.ANY),
        out_shape=jax.ShapeDtypeStruct((B, D), bf16),
        scratch_shapes=[
            pltpu.VMEM((B, D), bf16), pltpu.VMEM((B, D), bf16), pltpu.VMEM((F,), bf16), pltpu.VMEM((D,), bf16),
            pltpu.VMEM((D, H * DH), bf16), pltpu.VMEM((H * DH, D), bf16), pltpu.VMEM((F, D), bf16), pltpu.VMEM((F, D), bf16),
            pltpu.VMEM((D, 6 * D), bf16),
            pltpu.VMEM((NBUF, W, DH), bf16), pltpu.VMEM((NBUF, W, DH), bf16),
            pltpu.VMEM((H, 8, DH), f32), pltpu.VMEM((H, 8, DH), f32), pltpu.VMEM((B, D), bf16),
            pltpu.SemaphoreType.DMA((10,)), pltpu.SemaphoreType.DMA((NBUF,)), pltpu.SemaphoreType.DMA((NBUF,)),
        ],
        compiler_params=pltpu.CompilerParams(vmem_limit_bytes=100 * 1024 * 1024),
    )(x, c, B_b1, B_b2, k, v, A_wq, A_wo, B_w1.T, B_w2, w_mod)
    return out.reshape(B, 1, D)
```

```python
import functools
import jax
import jax.numpy as jnp
from jax import lax
import jax.experimental.pallas as pl
import jax.experimental.pallas.tpu as pltpu

B, D, H, S, DH, F = 4, 640, 32, 8192, 128, 1728
W = 2048
NT = W // 128
NU = B * H
NK, DK = 4, 3
NV, DV = 8, 7
EPS = 1e-5
bf16 = jnp.bfloat16
f32 = jnp.float32
NT_DIMS = (((1,), (1,)), ((), ()))
LOG2E = 1.4426950408889634
W2_GROUPS = (0, 512, 1024, 1408, 1664, 1728)
S_X, S_C, S_B1, S_B2, S_WMOD, S_WQ, S_WO, S_W1, S_OUT, S_W2 = range(10)
NSEM = S_W2 + len(W2_GROUPS) - 1


def _ln(x):
    m = jnp.mean(x, axis=-1, keepdims=True)
    xc = x - m
    v = jnp.mean(xc * xc, axis=-1, keepdims=True)
    return xc / jnp.sqrt(v + EPS)


def kernel(x_hbm, c_hbm, b1_hbm, b2_hbm, k_hbm, v_hbm, wq_hbm, wo_hbm, w1_hbm, w2_hbm, wmod_hbm,
           o_hbm,
           x_v, c_v, b1_v, b2_v, wq_v, wo_v, w1_v, w2_v, wmod_v, kvbuf, q_s, o_s, s_s, out_v, wsem, ksem, vsem):
    def cp(src, dst, i):
        return pltpu.make_async_copy(src, dst, wsem.at[i])

    def wait_all(buf, i):
        pltpu.make_async_copy(buf, buf, wsem.at[i]).wait()

    def rows(r, n):
        return pl.ds(pl.multiple_of(r * n, 8), n)

    def wq_piece(r, half):
        idx = (rows(r, 8), pl.ds(half * 2048, 2048))
        return cp(wq_hbm.at[idx], wq_v.at[idx], S_WQ)

    def wmod_piece(r, half):
        idx = (rows(r, 8), pl.ds(half * 1920, 1920))
        return cp(wmod_hbm.at[idx], wmod_v.at[idx], S_WMOD)

    def wo_piece(i):
        idx = (rows(i, 16), slice(None))
        return cp(wo_hbm.at[idx], wo_v.at[idx], S_WO)

    def w1_piece(i):
        idx = (rows(i, 24), slice(None))
        return cp(w1_hbm.at[idx], w1_v.at[idx], S_W1)

    def w2_piece(i):
        idx = (rows(i, 32), slice(None))
        g = sum(((i * 32 >= b).astype(jnp.int32) for b in W2_GROUPS[1:-1]), jnp.int32(0))
        return cp(w2_hbm.at[idx], w2_v.at[idx], S_W2 + g)

    def row_of(u):
        return (u & (B - 1)) * H + (u >> 2)

    def k_piece(u, t):
        slot = u & (NK - 1)
        return pltpu.make_async_copy(k_hbm.at[row_of(u), pl.ds(pl.multiple_of(S - W + t * 128, 128), 128), :],
                                     kvbuf.at[NV + slot, pl.ds(pl.multiple_of(t * 128, 128), 128), :], ksem.at[slot])

    def v_piece(u, t):
        slot = u & (NV - 1)
        return pltpu.make_async_copy(v_hbm.at[row_of(u), pl.ds(pl.multiple_of(S - W + t * 128, 128), 128), :],
                                     kvbuf.at[slot, pl.ds(pl.multiple_of(t * 128, 128), 128), :], vsem.at[slot])

    def k_wait(u):
        slot = u & (NK - 1)
        pltpu.make_async_copy(kvbuf.at[NV + slot], kvbuf.at[NV + slot], ksem.at[slot]).wait()

    def v_wait(u):
        slot = u & (NV - 1)
        pltpu.make_async_copy(kvbuf.at[slot], kvbuf.at[slot], vsem.at[slot]).wait()

    def loop(n, f):
        def body(i, c):
            f(i)
            return c
        lax.fori_loop(0, n, body, 0)

    small = [cp(x_hbm, x_v, S_X), cp(c_hbm, c_v, S_C), cp(b1_hbm, b1_v, S_B1), cp(b2_hbm, b2_v, S_B2)]

    def l0(i):
        wmod_piece(i, 0).start(priority=1)
        wmod_piece(i, 1).start(priority=1)
    loop(32, l0)
    for s in small:
        s.start(priority=0)

    def l1(i):
        wq_piece(i, 0).start(priority=0)
        wmod_piece(32 + i, 0).start(priority=1)
        wq_piece(i, 1).start(priority=0)
        wmod_piece(32 + i, 1).start(priority=1)
    loop(48, l1)

    def l2(i):
        wq_piece(48 + i, 0).start(priority=0)
        wo_piece(128 + 2 * i).start(priority=1)
        wq_piece(48 + i, 1).start(priority=0)
        wo_piece(128 + 2 * i + 1).start(priority=1)
    loop(32, l2)

    def l3(i):
        wo_piece(i).start(priority=0)
        wo_piece(192 + i).start(priority=1)
    loop(64, l3)

    for s in small:
        s.wait()
    wait_all(wmod_v, S_WMOD)
    cvec = c_v[...].astype(f32)
    sc = (cvec * jax.nn.sigmoid(cvec)).astype(bf16)
    mod = jnp.dot(sc, wmod_v[...], preferred_element_type=f32)
    sa, ca, ga, sb, cb, gb = [mod[:, i * D:(i + 1) * D] for i in range(6)]
    x = x_v[...].astype(f32)
    h1 = (_ln(x) * (1.0 + ca) + sa).astype(bf16)
    wait_all(wq_v, S_WQ)
    q = jnp.dot(h1, wq_v[...], preferred_element_type=f32)
    for h in range(H):
        q_s[h, 0:B, :] = q[:, h * DH:(h + 1) * DH]
        q_s[h, B:8, :] = jnp.zeros((8 - B, DH), f32)
    o_s[...] = jnp.zeros(o_s.shape, f32)

    def l4(i):
        wo_piece(64 + i).start(priority=0)
        v_piece(i >> 4, i & 15).start(priority=1)
    loop(64, l4)

    def l5(i):
        k_piece(i >> 4, i & 15).start(priority=0)
        v_piece(4 + (i >> 4), i & 15).start(priority=1)
    loop(48, l5)

    cexp = (DH ** -0.5) * LOG2E

    def qk_tile(qh, u, t):
        slot = u & (NK - 1)
        return lax.dot_general(qh, kvbuf[NV + slot, pl.ds(t * 128, 128), :], NT_DIMS, preferred_element_type=f32)

    k_wait(0)
    q0 = q_s[0].astype(bf16)
    mx = None
    for t in range(NT):
        st = qk_tile(q0, 0, t)
        s_s[0, t] = st
        mx = st if mx is None else jnp.maximum(mx, st)

    def make_body(issue, last=False):
        def body(u, mx):
            par = u & 1
            h = u >> 2
            b = u & 3
            m = jnp.max(mx, axis=-1, keepdims=True)
            if not last:
                k_wait(u + 1)
                qn = q_s[(u + 1) >> 2].astype(bf16)
            v_wait(u)
            vslot = u & (NV - 1)
            mxn = None
            lsum = None
            acc = None
            for t in range(NT):
                if not last:
                    st = qk_tile(qn, u + 1, t)
                    s_s[1 - par, t] = st
                    mxn = st if mxn is None else jnp.maximum(mxn, st)
                p = jnp.exp2((s_s[par, t] - m) * cexp)
                lsum = p if lsum is None else lsum + p
                pv = jnp.dot(p.astype(bf16), kvbuf[vslot, pl.ds(t * 128, 128), :], preferred_element_type=f32)
                acc = pv if acc is None else acc + pv
                issue(u, t)
            l = jnp.sum(lsum, axis=-1, keepdims=True)
            o = acc / l
            row = lax.broadcasted_iota(jnp.int32, (8, DH), 0)
            o_s[h] = jnp.where(row == b, o, o_s[h])
            return mxn if not last else mx
        return body

    def issue_main(u, t):
        k_piece(u + DK, t).start(priority=0)
        v_piece(u + DV, t).start(priority=1)

    def issue_mid(u, t):
        j = (u - (NU - DV)) * NT + t
        @pl.when(u + DK < NU)
        def _():
            k_piece(u + DK, t).start(priority=0)
        @pl.when(j < 54)
        def _():
            w2_piece(j).start(priority=1)
        if t < 12:
            @pl.when(u + DK >= NU)
            def _():
                jj = ((u - (NU - DK)) * 12 + t) * 3
                for i in range(3):
                    w1_piece(jj + i).start(priority=0)

    mx = lax.fori_loop(0, NU - DV, make_body(issue_main), mx)
    mx = lax.fori_loop(NU - DV, NU - 1, make_body(issue_mid), mx)
    make_body(lambda u, t: None, last=True)(jnp.int32(NU - 1), mx)

    wait_all(wo_v, S_WO)
    oall = jnp.concatenate([o_s[h] for h in range(H)], axis=1).astype(bf16)
    att = jnp.dot(oall, wo_v[...], preferred_element_type=f32)[0:B]
    x2 = x + ga * att
    h2 = (_ln(x2) * (1.0 + cb) + sb).astype(bf16)
    wait_all(w1_v, S_W1)
    hh = lax.dot_general(h2, w1_v[...], NT_DIMS, preferred_element_type=f32) + b1_v[...].astype(f32).reshape(1, F)
    hh = jax.nn.gelu(hh, approximate=True).astype(bf16)
    y = b2_v[...].astype(f32).reshape(1, D)
    for g in range(len(W2_GROUPS) - 1):
        r0, r1 = W2_GROUPS[g], W2_GROUPS[g + 1]
        wait_all(w2_v.at[pl.ds(r0, r1 - r0), :], S_W2 + g)
        y = y + jnp.dot(hh[:, r0:r1], w2_v[r0:r1, :], preferred_element_type=f32)
    out_v[...] = (x2 + gb * y).astype(bf16)
    co = cp(out_v, o_hbm, S_OUT)
    co.start(); co.wait()


@jax.jit
def pallas_adaLN_cond__sliding_block_cached__dense_activation_gelu__decode_kernel(A_x, A_k_cache, A_v_cache, A_wq, A_wo, B_x, B_w1, B_b1, B_w2, B_b2, c, w_mod):
    k = A_k_cache.reshape(B * H, S, DH)
    v = A_v_cache.reshape(B * H, S, DH)
    x = A_x.reshape(B, D)
    out = pl.pallas_call(
        kernel,
        in_specs=[pl.BlockSpec(memory_space=pl.ANY)] * 11,
        out_specs=pl.BlockSpec(memory_space=pl.ANY),
        out_shape=jax.ShapeDtypeStruct((B, D), bf16),
        scratch_shapes=[
            pltpu.VMEM((B, D), bf16), pltpu.VMEM((B, D), bf16), pltpu.VMEM((F,), bf16), pltpu.VMEM((D,), bf16),
            pltpu.VMEM((D, H * DH), bf16), pltpu.VMEM((H * DH, D), bf16), pltpu.VMEM((F, D), bf16), pltpu.VMEM((F, D), bf16),
            pltpu.VMEM((D, 6 * D), bf16),
            pltpu.VMEM((NK + NV, W, DH), bf16),
            pltpu.VMEM((H, 8, DH), f32), pltpu.VMEM((H, 8, DH), f32), pltpu.VMEM((2, NT, 8, 128), f32),
            pltpu.VMEM((B, D), bf16),
            pltpu.SemaphoreType.DMA((NSEM,)), pltpu.SemaphoreType.DMA((NK,)), pltpu.SemaphoreType.DMA((NV,)),
        ],
        compiler_params=pltpu.CompilerParams(vmem_limit_bytes=100 * 1024 * 1024, disable_bounds_checks=True),
    )(x, c, B_b1, B_b2, k, v, A_wq, A_wo, B_w1.T, B_w2, w_mod)
    return out.reshape(B, 1, D)
```

```python
import functools
import jax
import jax.numpy as jnp
from jax import lax
import jax.experimental.pallas as pl
import jax.experimental.pallas.tpu as pltpu

B, D, H, S, DH, F = 4, 640, 32, 8192, 128, 1728
W = 2048
NT = W // 128
NU = B * H
NK = 16
NV = 16
EPS = 1e-5
bf16 = jnp.bfloat16
f32 = jnp.float32
NT_DIMS = (((1,), (1,)), ((), ()))
LOG2E = 1.4426950408889634
S_X, S_C, S_B1, S_B2, S_WMOD, S_WQ, S_WO, S_OUT, S_W1, S_W2, S_K, S_V = 0, 1, 2, 3, 4, 5, 6, 7, 8, 24, 40, 56
NSEM = 72


def _ln(x):
    m = jnp.mean(x, axis=-1, keepdims=True)
    xc = x - m
    v = jnp.mean(xc * xc, axis=-1, keepdims=True)
    return xc / jnp.sqrt(v + EPS)


def kernel(cfg, x_hbm, c_hbm, b1_hbm, b2_hbm, k_hbm, v_hbm, wq_hbm, wo_hbm, w1_hbm, w2_hbm, wmod_hbm,
           o_hbm,
           x_v, c_v, b1_v, b2_v, wq_v, wo_v, w1_v, w2_v, wmod_v, kvbuf, q_s, att_s, s_s, out_v, sem):
    G = 4
    L = cfg.get("L", 7)
    assert L + G <= NV
    W1G = cfg.get("w1g", (0, 1728))
    W2G = cfg.get("w2g", (0, 1280, 1600, 1728))
    R1 = cfg.get("r1", 32)
    R2 = cfg.get("r2", 32)
    N1, N2 = F // R1, F // R2
    assert F % R1 == 0 and F % R2 == 0
    assert all(g % R1 == 0 for g in W1G) and all(g % R2 == 0 for g in W2G)
    P1, P2 = cfg.get("p1", 0), cfg.get("p2", 1)

    def cp(src, dst, i):
        return pltpu.make_async_copy(src, dst, sem.at[i])

    def wait_all(buf, i):
        pltpu.make_async_copy(buf, buf, sem.at[i]).wait()

    def rows(r, n):
        if isinstance(r, int):
            return pl.ds(r * n, n)
        return pl.ds(pl.multiple_of(r * n, 8), n)

    def wq_piece(i):
        idx = (rows(i >> 1, 8), pl.ds(pl.multiple_of((i & 1) * 2048, 128), 2048))
        return cp(wq_hbm.at[idx], wq_v.at[idx], S_WQ)

    def wmod_piece(i):
        idx = (rows(i >> 1, 8), pl.ds(pl.multiple_of((i & 1) * 1920, 128), 1920))
        return cp(wmod_hbm.at[idx], wmod_v.at[idx], S_WMOD)

    def wo_piece(i):
        idx = (rows(i, 32), slice(None))
        return cp(wo_hbm.at[idx], wo_v.at[idx], S_WO)

    def group(i, n, groups):
        if isinstance(i, int):
            return sum(int(i * n >= b) for b in groups[1:-1])
        return sum(((i * n >= b).astype(jnp.int32) for b in groups[1:-1]), jnp.int32(0))

    def w1_piece(i):
        idx = (rows(i, R1), slice(None))
        return cp(w1_hbm.at[idx], w1_v.at[idx], S_W1 + group(i, R1, W1G))

    def w2_piece(i):
        idx = (rows(i, R2), slice(None))
        return cp(w2_hbm.at[idx], w2_v.at[idx], S_W2 + group(i, R2, W2G))

    def row_of(u):
        return (u & (B - 1)) * H + (u >> 2)

    def tile(t, base=0):
        if isinstance(t, int):
            return pl.ds(base + t * 128, 128)
        return pl.ds(pl.multiple_of(base + t * 128, 128), 128)

    def k_piece(u, j):
        slot = u & (NK - 1)
        return cp(k_hbm.at[row_of(u), tile(j, S - W), :], kvbuf.at[NV + slot, tile(j), :], S_K + slot)

    def v_piece(u, j):
        slot = u & (NV - 1)
        return cp(v_hbm.at[row_of(u), tile(j, S - W), :], kvbuf.at[slot, tile(j), :], S_V + slot)

    def skew(v, t):
        e = t % G
        return v + L + (G - 1 - e), e * (NT // G) + t // G

    def k_wait(u):
        slot = u & (NK - 1)
        wait_all(kvbuf.at[NV + slot], S_K + slot)

    def v_wait(u):
        slot = u & (NV - 1)
        wait_all(kvbuf.at[slot], S_V + slot)

    def loop(n, f):
        def body(i, c):
            f(i)
            return c
        lax.fori_loop(0, n, body, 0)

    class Merge:
        def __init__(self, p0, p1):
            self.s = [[[f, 0, n] for f, n in p0], [[f, 0, n] for f, n in p1]]

        def take(self, p, n):
            f, s, e = self.s[p][0]
            self.s[p][0][1] += n
            if s + n == e:
                self.s[p].pop(0)
            return f, s

        def left(self, p):
            return self.s[p][0][2] - self.s[p][0][1]

        def single(self, p, cnt):
            while cnt > 0:
                n = min(cnt, self.left(p))
                f, s = self.take(p, n)
                loop(n, lambda i: f(s + i).start(priority=p))
                cnt -= n

        def pairs(self, cnt):
            while cnt > 0:
                n = min(cnt, self.left(0), self.left(1))
                f, s = self.take(0, n)
                g, r = self.take(1, n)

                def body(i):
                    f(s + i).start(priority=0)
                    g(r + i).start(priority=1)
                loop(n, body)
                cnt -= n

    small = [cp(x_hbm, x_v, S_X), cp(c_hbm, c_v, S_C), cp(b1_hbm, b1_v, S_B1), cp(b2_hbm, b2_v, S_B2)]
    mg = Merge([(wq_piece, 160), (wo_piece, 64)], [(wmod_piece, 160), (lambda i: wo_piece(64 + i), 64)])
    for s in small:
        s.start(priority=0)
    mg.pairs(224)
    assert not mg.s[0] and not mg.s[1]

    def kv_pro(lo, hi):
        def body(v, c):
            for t in range(NT):
                u, j = skew(v, t)

                @pl.when(u >= 0)
                def _():
                    k_piece(u, j).start(priority=0)
                    v_piece(u, j).start(priority=1)
            return c
        lax.fori_loop(lo, hi, body, 0)
    V0 = -(L + G - 1)
    VA = V0 + cfg.get("ua", 4)
    kv_pro(V0, VA)

    for s in small:
        s.wait()
    wait_all(wmod_v, S_WMOD)
    cvec = c_v[...].astype(f32)
    sc = (cvec * jax.nn.sigmoid(cvec)).astype(bf16)
    mod = jnp.dot(sc, wmod_v[...], preferred_element_type=f32)
    sa, ca, ga, sb, cb, gb = [mod[:, i * D:(i + 1) * D] for i in range(6)]
    x = x_v[...].astype(f32)
    h1 = (_ln(x) * (1.0 + ca) + sa).astype(bf16)
    wait_all(wq_v, S_WQ)
    q = jnp.dot(h1, wq_v[...], preferred_element_type=f32)
    for h in range(H):
        q_s[h, 0:B, :] = q[:, h * DH:(h + 1) * DH]
        q_s[h, B:8, :] = jnp.zeros((8 - B, DH), f32)
    att_s[...] = jnp.zeros(att_s.shape, f32)

    kv_pro(VA, 0)

    cexp = (DH ** -0.5) * LOG2E

    def qk_tile(qh, u, t):
        slot = u & (NK - 1)
        return lax.dot_general(qh, kvbuf[NV + slot, tile(t), :], NT_DIMS, preferred_element_type=f32)

    wait_all(wo_v, S_WO)
    k_wait(0)
    q0 = q_s[0].astype(bf16)
    mx = None
    for t in range(NT):
        st = qk_tile(q0, 0, t)
        s_s[0, t] = st
        mx = st if mx is None else jnp.maximum(mx, st)

    row = lax.broadcasted_iota(jnp.int32, (8, DH), 0)

    def finalize(u, acc, lsum):
        l = jnp.sum(lsum, axis=-1, keepdims=True)
        o = jnp.where(row == (u & 3), acc / l, 0.0).astype(bf16)
        h = jnp.maximum(u, 0) >> 2
        return jnp.dot(o, wo_v[tile(h), :], preferred_element_type=f32)

    def make_body(issue, last=False):
        def body(u, carry):
            mx, acc_p, lsum_p = carry
            par = u & 1
            m = jnp.max(mx, axis=-1, keepdims=True)
            if not last:
                k_wait(u + 1)
                qn = q_s[(u + 1) >> 2].astype(bf16)
            v_wait(u)
            if cfg.get("no_main"):
                for t in range(NT):
                    issue(u, t)
                return carry
            att_s[...] += finalize(u - 1, acc_p, lsum_p)
            vslot = u & (NV - 1)
            mxn = None
            lsum = None
            acc = None
            for t in range(NT):
                if not last:
                    st = qk_tile(qn, u + 1, t)
                    s_s[1 - par, t] = st
                    mxn = st if mxn is None else jnp.maximum(mxn, st)
                p = jnp.exp2((s_s[par, t] - m) * cexp)
                lsum = p if lsum is None else lsum + p
                pv = jnp.dot(p.astype(bf16), kvbuf[vslot, tile(t), :], preferred_element_type=f32)
                acc = pv if acc is None else acc + pv
                issue(u, t)
            return (mxn if not last else mx, acc, lsum)
        return body

    def issue_main(v, t):
        u, j = skew(v, t)
        k_piece(u, j).start(priority=0)
        v_piece(u, j).start(priority=1)

    VM = NU - (L + G - 1)
    free = [(v, t) for v in range(VM, NU - 1) for t in range(NT) if v + L + (G - 1 - t % G) >= NU]
    SK1 = cfg.get("skip1", cfg.get("skip", 0))
    SK2 = cfg.get("skip2", cfg.get("skip", 0))
    assert SK1 + N1 <= len(free) and SK2 + N2 <= len(free), (N1, N2, len(free))
    base = {v: next(i for i, (vv, _) in enumerate(free) if vv == v) for v in range(VM, NU - 1)}

    def issue_mid(v, t):
        u, j = skew(v, t)

        @pl.when(u < NU)
        def _():
            k_piece(u, j).start(priority=0)
            v_piece(u, j).start(priority=1)
        d = v - VM
        nf = jnp.minimum(d + 1, G)
        before = jnp.where(d < G, d * (d + 1) // 2 * (NT // G), (G * (G - 1) // 2) * (NT // G) + (d - (G - 1)) * NT)
        idx = before + (t // G) * nf + (t % G)

        @pl.when(jnp.logical_and(u >= NU, jnp.logical_and(idx >= SK1, idx < SK1 + N1)))
        def _():
            w1_piece(idx - SK1).start(priority=0)

        @pl.when(jnp.logical_and(u >= NU, jnp.logical_and(idx >= SK2, idx < SK2 + N2)))
        def _():
            w2_piece(idx - SK2).start(priority=1)

    for i, (v, t) in enumerate(free):
        d = v - VM
        nf = min(d + 1, G)
        before = d * (d + 1) // 2 * (NT // G) if d < G else (G * (G - 1) // 2) * (NT // G) + (d - (G - 1)) * NT
        assert before + (t // G) * nf + (t % G) == i, (i, v, t)

    carry = (mx, jnp.zeros((8, DH), f32), jnp.ones((8, DH), f32))
    carry = lax.fori_loop(0, VM, make_body(issue_main), carry)
    carry = lax.fori_loop(VM, NU - 1, make_body(issue_mid), carry)
    _, acc, lsum = make_body(lambda u, t: None, last=True)(jnp.int32(NU - 1), carry)
    att = (att_s[...] + finalize(jnp.int32(NU - 1), acc, lsum))[0:B]

    x2 = x + ga * att
    if cfg.get("no_tail"):
        for g in range(len(W1G) - 1):
            wait_all(w1_v.at[pl.ds(W1G[g], W1G[g + 1] - W1G[g]), :], S_W1 + g)
        for g in range(len(W2G) - 1):
            wait_all(w2_v.at[pl.ds(W2G[g], W2G[g + 1] - W2G[g]), :], S_W2 + g)
        out_v[...] = x2.astype(bf16)
        co = cp(out_v, o_hbm, S_OUT)
        co.start(); co.wait()
        return
    h2 = (_ln(x2) * (1.0 + cb) + sb).astype(bf16)
    b1 = b1_v[...].astype(f32).reshape(1, F)
    hhs = []
    for g in range(len(W1G) - 1):
        r0, r1 = W1G[g], W1G[g + 1]
        wait_all(w1_v.at[pl.ds(r0, r1 - r0), :], S_W1 + g)
        hh = lax.dot_general(h2, w1_v[r0:r1, :], NT_DIMS, preferred_element_type=f32) + b1[:, r0:r1]
        hhs.append(jax.nn.gelu(hh, approximate=True).astype(bf16))
    hh = hhs[0] if len(hhs) == 1 else jnp.concatenate(hhs, axis=1)
    y = b2_v[...].astype(f32).reshape(1, D)
    for g in range(len(W2G) - 1):
        r0, r1 = W2G[g], W2G[g + 1]
        wait_all(w2_v.at[pl.ds(r0, r1 - r0), :], S_W2 + g)
        y = y + jnp.dot(hh[:, r0:r1], w2_v[r0:r1, :], preferred_element_type=f32)
    out_v[...] = (x2 + gb * y).astype(bf16)
    co = cp(out_v, o_hbm, S_OUT)
    co.start(); co.wait()


CFG = dict(L=5, skip1=0, skip2=12)


@jax.jit
def pallas_adaLN_cond__sliding_block_cached__dense_activation_gelu__decode_kernel(A_x, A_k_cache, A_v_cache, A_wq, A_wo, B_x, B_w1, B_b1, B_w2, B_b2, c, w_mod):
    k = A_k_cache.reshape(B * H, S, DH)
    v = A_v_cache.reshape(B * H, S, DH)
    x = A_x.reshape(B, D)
    out = pl.pallas_call(
        functools.partial(kernel, CFG),
        in_specs=[pl.BlockSpec(memory_space=pl.ANY)] * 11,
        out_specs=pl.BlockSpec(memory_space=pl.ANY),
        out_shape=jax.ShapeDtypeStruct((B, D), bf16),
        scratch_shapes=[
            pltpu.VMEM((B, D), bf16), pltpu.VMEM((B, D), bf16), pltpu.VMEM((F,), bf16), pltpu.VMEM((D,), bf16),
            pltpu.VMEM((D, H * DH), bf16), pltpu.VMEM((H * DH, D), bf16), pltpu.VMEM((F, D), bf16), pltpu.VMEM((F, D), bf16),
            pltpu.VMEM((D, 6 * D), bf16),
            pltpu.VMEM((NK + NV, W, DH), bf16),
            pltpu.VMEM((H, 8, DH), f32), pltpu.VMEM((8, D), f32), pltpu.VMEM((2, NT, 8, 128), f32),
            pltpu.VMEM((B, D), bf16),
            pltpu.SemaphoreType.DMA((NSEM,)),
        ],
        compiler_params=pltpu.CompilerParams(vmem_limit_bytes=100 * 1024 * 1024, disable_bounds_checks=True,
                                             disable_semaphore_checks=True),
    )(x, c, B_b1, B_b2, k, v, A_wq, A_wo, B_w1.T, B_w2, w_mod)
    return out.reshape(B, 1, D)
```

```python
import functools
import jax
import jax.numpy as jnp
from jax import lax
import jax.experimental.pallas as pl
import jax.experimental.pallas.tpu as pltpu

B, D, H, S, DH, F = 4, 640, 32, 8192, 128, 1728
W = 2048
NT = W // 128
NU = B * H
NK = 16
NV = 16
G = 4
EPS = 1e-5
bf16 = jnp.bfloat16
f32 = jnp.float32
NT_DIMS = (((1,), (1,)), ((), ()))
LOG2E = 1.4426950408889634
S_X, S_C, S_B1, S_B2, S_WM, S_WQ, S_WO, S_OUT, S_W1, S_W2, S_K, S_V = 0, 1, 2, 3, 4, 5, 6, 7, 8, 16, 24, 40
NSEM = 56
PT = 16
N_WQ, N_WO, N_WM, N_W1, N_W2 = 2560, 2560, 2400, 1080, 1080


def _ln(x):
    m = jnp.mean(x, axis=-1, keepdims=True)
    xc = x - m
    v = jnp.mean(xc * xc, axis=-1, keepdims=True)
    return xc / jnp.sqrt(v + EPS)


def _cols(w_v, lo, nslab, ct):
    blk = w_v[pl.ds(lo, nslab * ct)].reshape(nslab, ct, 8, 128)
    return [blk[:, c].reshape(nslab * 8, 128) for c in range(ct)]


def kernel(cfg, x_hbm, c_hbm, b1_hbm, b2_hbm, k_hbm, v_hbm, wq_hbm, wo_hbm, w1_hbm, w2_hbm, wm_hbm,
           o_hbm,
           x_v, c_v, b1_v, b2_v, wq_v, wo_v, w1_v, w2_v, wm_v, kvbuf, q_s, att_s, s_s, out_v, sem):
    L = cfg.get("L", 5)
    assert L + G <= NV
    PH_WM, PH_W1, PH_W2 = cfg.get("ph", (7, 13, 3))
    W2R = cfg.get("w2r", (0, 1280, 1600, 1728))
    W2B = [0] + [-(-(r // 8 * 5 - PH_W2) // PT) * PT + PH_W2 for r in W2R[1:-1]] + [N_W2]

    def cp(src, dst, i):
        return pltpu.make_async_copy(src, dst, sem.at[i])

    def wait_all(buf, i):
        pltpu.make_async_copy(buf, buf, sem.at[i]).wait()

    def wpiece(hbm, vm, s):
        def f(lo, n=PT):
            return cp(hbm.at[pl.ds(lo, n)], vm.at[pl.ds(lo, n)], s)
        return f
    wq_p = wpiece(wq_hbm, wq_v, S_WQ)
    wo_p = wpiece(wo_hbm, wo_v, S_WO)
    wm_p = wpiece(wm_hbm, wm_v, S_WM)
    w1_p = wpiece(w1_hbm, w1_v, S_W1)

    def w2_p(lo, n=PT):
        if isinstance(lo, int):
            g = sum(int(lo >= b) for b in W2B[1:-1])
        else:
            g = sum(((lo >= b).astype(jnp.int32) for b in W2B[1:-1]), jnp.int32(0))
        return cp(w2_hbm.at[pl.ds(lo, n)], w2_v.at[pl.ds(lo, n)], S_W2 + g)

    def row_of(u):
        return (u & (B - 1)) * H + (u >> 2)

    def tile(t, base=0):
        return pl.ds(base + t * 128, 128)

    PH_KV = cfg.get("phkv", 62)
    KVB = [0] + [PH_KV + 64 * i for i in range(NT - 1)] + [W // 2]

    def k_piece(u, j):
        slot = u & (NK - 1)
        n = KVB[j + 1] - KVB[j]
        return cp(k_hbm.at[row_of(u), pl.ds((S - W) // 2 + KVB[j], n)], kvbuf.at[NV + slot, pl.ds(KVB[j], n)], S_K + slot)

    def v_piece(u, j):
        slot = u & (NV - 1)
        n = KVB[j + 1] - KVB[j]
        return cp(v_hbm.at[row_of(u), pl.ds((S - W) // 2 + KVB[j], n)], kvbuf.at[slot, pl.ds(KVB[j], n)], S_V + slot)

    kv32 = kvbuf.bitcast(jnp.uint32).at[:, :, 0]

    def kv_tile(slot, t):
        return pltpu.bitcast(kv32[slot, pl.ds(t * 64, 64), :], bf16)

    def skew(v, t):
        e = t % G
        return v + L + (G - 1 - e), e * (NT // G) + t // G

    def k_wait(u):
        slot = u & (NK - 1)
        wait_all(kvbuf.at[NV + slot], S_K + slot)

    def v_wait(u):
        slot = u & (NV - 1)
        wait_all(kvbuf.at[slot], S_V + slot)

    def loop(lo, hi, f):
        def body(i, c):
            f(i)
            return c
        lax.fori_loop(lo, hi, body, 0)

    small = [cp(x_hbm, x_v, S_X), cp(c_hbm, c_v, S_C), cp(b1_hbm, b1_v, S_B1), cp(b2_hbm, b2_v, S_B2)]
    HQ = N_WQ // 2
    NM0 = 75
    M1 = PH_WM + NM0 * PT
    NM1 = (N_WM - M1) // PT

    def pro3(i):
        wq_p(i * PT).start(priority=0)
        wq_p(HQ + i * PT).start(priority=1)
        wo_p(i * PT).start(priority=0)
        wo_p(HQ + i * PT).start(priority=1)
        wm_p(PH_WM + i * PT).start(priority=0)
        wm_p(M1 + i * PT).start(priority=1)

    def pro2(i):
        wq_p(i * PT).start(priority=0)
        wq_p(HQ + i * PT).start(priority=1)
        wo_p(i * PT).start(priority=0)
        wo_p(HQ + i * PT).start(priority=1)
    assert NM1 == NM0 - 1
    loop(0, NM1, pro3)
    for s in small:
        s.start(priority=0)
    wm_p(PH_WM + NM1 * PT).start(priority=0)
    wm_p(M1 + NM1 * PT, N_WM - (M1 + NM1 * PT)).start(priority=1)
    wm_p(0, PH_WM).start(priority=0)
    loop(NM1, HQ // PT, pro2)

    def kv_pro(lo, hi):
        def body(v):
            for t in range(NT):
                u, j = skew(v, t)

                @pl.when(u >= 0)
                def _():
                    k_piece(u, j).start(priority=0)
                    v_piece(u, j).start(priority=1)
        loop(lo, hi, body)
    V0 = -(L + G - 1)
    VA = min(0, V0 + cfg.get("ua", 6))
    kv_pro(V0, VA)

    for s in small:
        s.wait()
    wait_all(wm_v, S_WM)
    cvec = c_v[...].astype(f32)
    sc = (cvec * jax.nn.sigmoid(cvec)).astype(bf16)
    x = x_v[...].astype(f32)
    if cfg.get("no_pro"):
        mod = jnp.concatenate([cvec] * 6, axis=1)
    else:
        mod = jnp.concatenate([jnp.dot(sc, wc, preferred_element_type=f32) for wc in _cols(wm_v, 0, 80, 30)], axis=1)
    sa, ca, ga, sb, cb, gb = [mod[:, i * D:(i + 1) * D] for i in range(6)]
    h1 = (_ln(x) * (1.0 + ca) + sa).astype(bf16)
    wait_all(wq_v, S_WQ)
    if cfg.get("no_pro"):
        for h in range(H):
            q_s[h, 0:B, :] = x[:, 0:128]
    else:
        for h, wc in enumerate(_cols(wq_v, 0, 80, 32)):
            q_s[h, 0:B, :] = jnp.dot(h1, wc, preferred_element_type=f32)
    q_s[:, B:8, :] = jnp.zeros((H, 8 - B, DH), f32)
    att_s[...] = jnp.zeros(att_s.shape, f32)

    if VA < 0:
        kv_pro(VA, 0)

    cexp = (DH ** -0.5) * LOG2E

    def qk_tile(qh, u, t):
        slot = u & (NK - 1)
        return lax.dot_general(qh, kv_tile(NV + slot, t), NT_DIMS, preferred_element_type=f32)

    wait_all(wo_v, S_WO)
    k_wait(0)
    q0 = q_s[0].astype(bf16)
    mx = None
    for t in range(NT):
        st = qk_tile(q0, 0, t)
        s_s[0, t] = st
        mx = st if mx is None else jnp.maximum(mx, st)

    row = lax.broadcasted_iota(jnp.int32, (8, DH), 0)

    def finalize(u, acc, lsum):
        l = jnp.sum(lsum, axis=-1, keepdims=True)
        o = jnp.where(row == (u & 3), acc / l, 0.0).astype(bf16)
        h = jnp.maximum(u, 0) >> 2
        return jnp.concatenate([jnp.dot(o, wc, preferred_element_type=f32) for wc in _cols(wo_v, h * 80, 16, 5)], axis=1)

    def make_body(issue, last=False):
        def body(u, carry):
            mx, acc_p, lsum_p = carry
            par = u & 1
            m = jnp.max(mx, axis=-1, keepdims=True)
            if not last:
                k_wait(u + 1)
                qn = q_s[(u + 1) >> 2].astype(bf16)
            v_wait(u)
            if cfg.get("no_main"):
                for t in range(NT):
                    issue(u, t)
                return carry
            att_s[...] += finalize(u - 1, acc_p, lsum_p)
            vslot = u & (NV - 1)
            mxn = None
            lsum = None
            acc = None
            for t in range(NT):
                if not last:
                    st = qk_tile(qn, u + 1, t)
                    s_s[1 - par, t] = st
                    mxn = st if mxn is None else jnp.maximum(mxn, st)
                p = jnp.exp2((s_s[par, t] - m) * cexp)
                lsum = p if lsum is None else lsum + p
                pv = jnp.dot(p.astype(bf16), kv_tile(vslot, t), preferred_element_type=f32)
                acc = pv if acc is None else acc + pv
                issue(u, t)
            return (mxn if not last else mx, acc, lsum)
        return body

    def issue_main(v, t):
        u, j = skew(v, t)
        k_piece(u, j).start(priority=0)
        v_piece(u, j).start(priority=1)

    VM = NU - (L + G - 1)
    free = [(v, t) for v in range(VM, NU - 1) for t in range(NT) if v + L + (G - 1 - t % G) >= NU]
    SK1, SK2 = cfg.get("skip1", 0), cfg.get("skip2", 12)
    N1 = (N_W1 - PH_W1) // PT
    N2 = (N_W2 - PH_W2) // PT
    assert SK1 + N1 <= len(free) and SK2 + N2 <= len(free), (N1, N2, len(free))

    def slot_index(d, t, mn, sel):
        nf = mn(d + 1, G)
        before = sel(d < G, d * (d + 1) // 2 * (NT // G), (G * (G - 1) // 2) * (NT // G) + (d - (G - 1)) * NT)
        return before + (t // G) * nf + (t % G)
    for i, (v, t) in enumerate(free):
        assert slot_index(v - VM, t, min, lambda c, a, b: a if c else b) == i

    def issue_mid(v, t):
        u, j = skew(v, t)

        @pl.when(u < NU)
        def _():
            k_piece(u, j).start(priority=0)
            v_piece(u, j).start(priority=1)
        idx = slot_index(v - VM, t, jnp.minimum, jnp.where)

        @pl.when(jnp.logical_and(u >= NU, jnp.logical_and(idx >= SK1, idx < SK1 + N1)))
        def _():
            w1_p(PH_W1 + (idx - SK1) * PT).start(priority=0)

        @pl.when(jnp.logical_and(u >= NU, jnp.logical_and(idx >= SK2, idx < SK2 + N2)))
        def _():
            w2_p(PH_W2 + (idx - SK2) * PT).start(priority=1)

        @pl.when(jnp.logical_and(u >= NU, idx == SK2 + N2 - 1))
        def _():
            w2_p(PH_W2 + N2 * PT, N_W2 - PH_W2 - N2 * PT).start(priority=1)

    carry = (mx, jnp.zeros((8, DH), f32), jnp.ones((8, DH), f32))
    carry = lax.fori_loop(0, VM, make_body(issue_main), carry)
    w1_p(0, PH_W1).start(priority=0)
    w1_p(PH_W1 + N1 * PT, N_W1 - PH_W1 - N1 * PT).start(priority=0)
    w2_p(0, PH_W2).start(priority=1)
    carry = lax.fori_loop(VM, NU - 1, make_body(issue_mid), carry)
    _, acc, lsum = make_body(lambda u, t: None, last=True)(jnp.int32(NU - 1), carry)
    att = (att_s[...] + finalize(jnp.int32(NU - 1), acc, lsum))[0:B]

    x2 = x + ga * att
    if cfg.get("no_tail"):
        wait_all(w1_v, S_W1)
        for g in range(len(W2B) - 1):
            wait_all(w2_v.at[pl.ds(W2B[g], W2B[g + 1] - W2B[g])], S_W2 + g)
        out_v[...] = x2.astype(bf16)
        co = cp(out_v, o_hbm, S_OUT)
        co.start(); co.wait()
        return
    h2 = (_ln(x2) * (1.0 + cb) + sb).astype(bf16)
    wait_all(w1_v, S_W1)
    hh = b1_v[...].astype(f32).reshape(1, F)
    for c, wc in enumerate(_cols(w1_v, 0, F // 8, 5)):
        hh = hh + lax.dot_general(h2[:, c * 128:(c + 1) * 128], wc, NT_DIMS, preferred_element_type=f32)
    hh = jax.nn.gelu(hh, approximate=True).astype(bf16)
    y = b2_v[...].astype(f32).reshape(1, D)
    for g in range(len(W2R) - 1):
        r0, r1 = W2R[g], W2R[g + 1]
        wait_all(w2_v.at[pl.ds(W2B[g], W2B[g + 1] - W2B[g])], S_W2 + g)
        y = y + jnp.concatenate([jnp.dot(hh[:, r0:r1], wc, preferred_element_type=f32)
                                 for wc in _cols(w2_v, r0 // 8 * 5, (r1 - r0) // 8, 5)], axis=1)
    out_v[...] = (x2 + gb * y).astype(bf16)
    co = cp(out_v, o_hbm, S_OUT)
    co.start(); co.wait()


def _tiles(w):
    r, c = w.shape
    return w.reshape(r // 8, 8, c // 128, 128).transpose(0, 2, 1, 3).reshape(-1, 8, 128)


CFG = dict()


@jax.jit
def pallas_adaLN_cond__sliding_block_cached__dense_activation_gelu__decode_kernel(A_x, A_k_cache, A_v_cache, A_wq, A_wo, B_x, B_w1, B_b1, B_w2, B_b2, c, w_mod):
    k = A_k_cache.reshape(B * H, S // 2, 2, DH)
    v = A_v_cache.reshape(B * H, S // 2, 2, DH)
    x = A_x.reshape(B, D)
    out = pl.pallas_call(
        functools.partial(kernel, CFG),
        in_specs=[pl.BlockSpec(memory_space=pl.ANY)] * 11,
        out_specs=pl.BlockSpec(memory_space=pl.ANY),
        out_shape=jax.ShapeDtypeStruct((B, D), bf16),
        scratch_shapes=[
            pltpu.VMEM((B, D), bf16), pltpu.VMEM((B, D), bf16), pltpu.VMEM((F,), bf16), pltpu.VMEM((D,), bf16),
            pltpu.VMEM((N_WQ, 8, 128), bf16), pltpu.VMEM((N_WO, 8, 128), bf16), pltpu.VMEM((N_W1, 8, 128), bf16),
            pltpu.VMEM((N_W2, 8, 128), bf16), pltpu.VMEM((N_WM, 8, 128), bf16),
            pltpu.VMEM((NK + NV, W // 2, 2, DH), bf16),
            pltpu.VMEM((H, 8, DH), f32), pltpu.VMEM((8, D), f32), pltpu.VMEM((2, NT, 8, 128), f32),
            pltpu.VMEM((B, D), bf16),
            pltpu.SemaphoreType.DMA((NSEM,)),
        ],
        compiler_params=pltpu.CompilerParams(vmem_limit_bytes=100 * 1024 * 1024, disable_bounds_checks=True,
                                             disable_semaphore_checks=True),
    )(x, c, B_b1, B_b2, k, v, _tiles(A_wq), _tiles(A_wo), _tiles(B_w1.T), _tiles(B_w2), _tiles(w_mod))
    return out.reshape(B, 1, D)
```

```python
import functools

import jax
import jax.numpy as jnp
from jax import lax
import jax.experimental.pallas as pl
import jax.experimental.pallas.tpu as pltpu

B, D, H, S, DH, F = 4, 640, 32, 8192, 128, 1728
W = min(4096, max(256, S // 4))
NT = W // 128
NU = B * H
NSLOT = 16
G = 4
EPS = 1e-5
LOG2E = 1.4426950408889634
bf16 = jnp.bfloat16
f32 = jnp.float32
NT_DIMS = (((1,), (1,)), ((), ()))

PT = 16
CT = D // 128
N_WQ, N_WO, N_WM, N_W1, N_W2 = D * H * DH // 1024, H * DH * D // 1024, D * 6 * D // 1024, F * D // 1024, F * D // 1024

S_X, S_C, S_B1, S_B2, S_WM, S_WQ, S_WO, S_OUT, S_W1, S_W2, S_K, S_V = 0, 1, 2, 3, 4, 5, 6, 7, 8, 9, 16, 32
NSEM = S_V + NSLOT


def _ln(x):
    m = jnp.mean(x, axis=-1, keepdims=True)
    xc = x - m
    v = jnp.mean(xc * xc, axis=-1, keepdims=True)
    return xc / jnp.sqrt(v + EPS)


def _cols(w_v, lo, nslab, ct):
    blk = w_v[pl.ds(lo, nslab * ct)].reshape(nslab, ct, 8, 128)
    return [blk[:, c].reshape(nslab * 8, 128) for c in range(ct)]


def _matmul_cols(a, cols):
    return jnp.concatenate([jnp.dot(a, wc, preferred_element_type=f32) for wc in cols], axis=1)


def kernel(cfg, x_hbm, c_hbm, b1_hbm, b2_hbm, k_hbm, v_hbm, wq_hbm, wo_hbm, w1_hbm, w2_hbm, wm_hbm,
           o_hbm,
           x_v, c_v, b1_v, b2_v, wq_v, wo_v, w1_v, w2_v, wm_v, kvbuf, q_s, att_s, s_s, out_v, sem):
    L = cfg.get("L", 5)
    UA = cfg.get("ua", 6)
    SK1, SK2 = cfg.get("skip1", 0), cfg.get("skip2", 12)
    PH_KV, PH_WM, PH_W1, PH_W2 = cfg.get("ph", (62, 7, 13, 3))
    assert 2 <= L and L + G <= NSLOT

    def cp(src, dst, i):
        return pltpu.make_async_copy(src, dst, sem.at[i])

    def wait_all(buf, i):
        pltpu.make_async_copy(buf, buf, sem.at[i]).wait()

    def loop(lo, hi, f):
        def body(i, c):
            f(i)
            return c
        lax.fori_loop(lo, hi, body, 0)

    def wpiece(hbm, vm, s0):
        def start(lo, prio, n=PT, g=0):
            cp(hbm.at[pl.ds(lo, n)], vm.at[pl.ds(lo, n)], s0 + g).start(priority=prio)
        return start
    wq_p = wpiece(wq_hbm, wq_v, S_WQ)
    wo_p = wpiece(wo_hbm, wo_v, S_WO)
    wm_p = wpiece(wm_hbm, wm_v, S_WM)
    w1_p = wpiece(w1_hbm, w1_v, S_W1)
    w2_p = wpiece(w2_hbm, w2_v, S_W2)

    KVB = [0] + [PH_KV + 64 * i for i in range(NT - 1)] + [W // 2]

    def kv_start(u, j):
        row = (u & (B - 1)) * H + (u >> 2)
        slot = u & (NSLOT - 1)
        n = KVB[j + 1] - KVB[j]
        src = pl.ds((S - W) // 2 + KVB[j], n)
        dst = pl.ds(KVB[j], n)
        cp(k_hbm.at[row, src], kvbuf.at[NSLOT + slot, dst], S_K + slot).start(priority=0)
        cp(v_hbm.at[row, src], kvbuf.at[slot, dst], S_V + slot).start(priority=1)

    def skew(v, t):
        e = t % G
        return v + L + (G - 1 - e), e * (NT // G) + t // G

    def k_wait(u):
        slot = u & (NSLOT - 1)
        wait_all(kvbuf.at[NSLOT + slot], S_K + slot)

    def v_wait(u):
        slot = u & (NSLOT - 1)
        wait_all(kvbuf.at[slot], S_V + slot)

    kv32 = kvbuf.bitcast(jnp.uint32).at[:, :, 0]

    def kv_tile(slot, t):
        return pltpu.bitcast(kv32[slot, pl.ds(t * 64, 64), :], bf16)

    small = [cp(x_hbm, x_v, S_X), cp(c_hbm, c_v, S_C), cp(b1_hbm, b1_v, S_B1), cp(b2_hbm, b2_v, S_B2)]
    HQ = N_WQ // 2
    NM = (N_WM - PH_WM) // PT // 2
    M1 = PH_WM + (NM + 1) * PT
    assert N_WO == N_WQ and HQ % PT == 0 and 0 < N_WM - (M1 + NM * PT) <= PT and NM <= HQ // PT

    def pro2(i):
        wq_p(i * PT, 0)
        wq_p(HQ + i * PT, 1)
        wo_p(i * PT, 0)
        wo_p(HQ + i * PT, 1)

    def pro3(i):
        pro2(i)
        wm_p(PH_WM + i * PT, 0)
        wm_p(M1 + i * PT, 1)
    loop(0, NM, pro3)
    for s in small:
        s.start(priority=0)
    wm_p(PH_WM + NM * PT, 0)
    wm_p(M1 + NM * PT, 1, N_WM - (M1 + NM * PT))
    wm_p(0, 0, PH_WM)
    loop(NM, HQ // PT, pro2)

    def kv_prologue(v):
        for t in range(NT):
            u, j = skew(v, t)
            pl.when(u >= 0)(functools.partial(kv_start, u, j))
    V0 = -(L + G - 1)
    VA = min(0, V0 + UA)
    loop(V0, VA, kv_prologue)

    for s in small:
        s.wait()
    wait_all(wm_v, S_WM)
    cvec = c_v[...].astype(f32)
    x = x_v[...].astype(f32)
    mod = _matmul_cols((cvec * jax.nn.sigmoid(cvec)).astype(bf16), _cols(wm_v, 0, D // 8, 6 * CT))
    sa, ca, ga, sb, cb, gb = [mod[:, i * D:(i + 1) * D] for i in range(6)]
    h1 = (_ln(x) * (1.0 + ca) + sa).astype(bf16)
    wait_all(wq_v, S_WQ)
    for h, wc in enumerate(_cols(wq_v, 0, D // 8, H)):
        q_s[h, 0:B, :] = jnp.dot(h1, wc, preferred_element_type=f32)
    q_s[:, B:8, :] = jnp.zeros((H, 8 - B, DH), f32)
    att_s[...] = jnp.zeros(att_s.shape, f32)
    if VA < 0:
        loop(VA, 0, kv_prologue)

    cexp = (DH ** -0.5) * LOG2E
    row = lax.broadcasted_iota(jnp.int32, (8, DH), 0)

    def qk_tile(qh, u, t):
        return lax.dot_general(qh, kv_tile(NSLOT + (u & (NSLOT - 1)), t), NT_DIMS, preferred_element_type=f32)

    def project(u, acc, lsum):
        l = jnp.sum(lsum, axis=-1, keepdims=True)
        o = jnp.where(row == (u & (B - 1)), acc / l, 0.0).astype(bf16)
        h = jnp.maximum(u, 0) >> 2
        return _matmul_cols(o, _cols(wo_v, h * (DH // 8 * CT), DH // 8, CT))

    def make_body(issue, last=False):
        def body(u, carry):
            mx, acc_p, lsum_p = carry
            par = u & 1
            m = jnp.max(mx, axis=-1, keepdims=True)
            if not last:
                k_wait(u + 1)
                qn = q_s[(u + 1) >> 2].astype(bf16)
            v_wait(u)
            att_s[...] += project(u - 1, acc_p, lsum_p)
            mxn = lsum = acc = None
            for t in range(NT):
                if not last:
                    st = qk_tile(qn, u + 1, t)
                    s_s[1 - par, t] = st
                    mxn = st if mxn is None else jnp.maximum(mxn, st)
                p = jnp.exp2((s_s[par, t] - m) * cexp)
                lsum = p if lsum is None else lsum + p
                pv = jnp.dot(p.astype(bf16), kv_tile(u & (NSLOT - 1), t), preferred_element_type=f32)
                acc = pv if acc is None else acc + pv
                issue(u, t)
            return (mx if last else mxn), acc, lsum
        return body

    wait_all(wo_v, S_WO)
    k_wait(0)
    q0 = q_s[0].astype(bf16)
    mx = None
    for t in range(NT):
        st = qk_tile(q0, 0, t)
        s_s[0, t] = st
        mx = st if mx is None else jnp.maximum(mx, st)

    VM = NU - (L + G - 1)
    free = [(v, t) for v in range(VM, NU - 1) for t in range(NT) if skew(v, t)[0] >= NU]
    N1 = (N_W1 - PH_W1) // PT
    N2 = (N_W2 - PH_W2) // PT
    NS2, RB2 = cfg.get("ns2", 20), cfg.get("rb2", 15)
    assert SK1 + N1 <= len(free) and SK2 + N2 <= len(free) and N1 >= 64 and N2 >= 3 * NS2
    assert all((i * 43) >> 7 == i // 3 for i in range(N2))

    def slot_index(d, t, minimum, where):
        nfree = minimum(d + 1, G)
        before = where(d < G, d * (d + 1) // 2 * (NT // G), (G * (G - 1) // 2) * (NT // G) + (d - (G - 1)) * NT)
        return before + (t // G) * nfree + (t % G)
    for i, (v, t) in enumerate(free):
        assert slot_index(v - VM, t, min, lambda c, a, b: a if c else b) == i

    W2B = [0] + [PH_W2 + (s * NS2 + o) * PT for s in range(3) for o in (RB2, NS2)] + [N_W2]
    W2G = [0, 1, 0, 1, 0, 1, 2]
    W2R = [[], [], []]
    for r in range(0, F, 128):
        r1 = min(r + 128, F)
        g = max(W2G[i] for i in range(7) if W2B[i] < r1 // 8 * CT and W2B[i + 1] > r // 8 * CT)
        if W2R[g] and W2R[g][-1][1] == r:
            W2R[g][-1][1] = r1
        else:
            W2R[g].append([r, r1])

    def issue_main(v, t):
        kv_start(*skew(v, t))

    def issue_end(v, t):
        u, j = skew(v, t)
        pl.when(u < NU)(functools.partial(kv_start, u, j))
        idx = slot_index(v - VM, t, jnp.minimum, jnp.where)

        @pl.when(jnp.logical_and(u >= NU, jnp.logical_and(idx >= SK1, idx < SK1 + N1)))
        def _():
            i = idx - SK1
            w1_p(PH_W1 + jnp.where(i < 64, (i & 3) * 16 + (i >> 2), i) * PT, 0)

        @pl.when(jnp.logical_and(u >= NU, jnp.logical_and(idx >= SK2, idx < SK2 + N2)))
        def _():
            i = idx - SK2
            rnd = (i * 43) >> 7
            rr = i < 3 * NS2
            st = i - 3 * rnd
            w2_p(PH_W2 + jnp.where(rr, st * NS2 + rnd, i) * PT, 1,
                 g=jnp.where(rr, 2 * st + (rnd >= RB2).astype(jnp.int32), 6))

        @pl.when(jnp.logical_and(u >= NU, idx == SK2 + N2 - 1))
        def _():
            w2_p(PH_W2 + N2 * PT, 1, N_W2 - PH_W2 - N2 * PT, g=6)

    carry = (mx, jnp.zeros((8, DH), f32), jnp.ones((8, DH), f32))
    carry = lax.fori_loop(0, VM, make_body(issue_main), carry)
    w1_p(0, 0, PH_W1)
    w1_p(PH_W1 + N1 * PT, 0, N_W1 - PH_W1 - N1 * PT)
    w2_p(0, 1, PH_W2)
    carry = lax.fori_loop(VM, NU - 1, make_body(issue_end), carry)
    _, acc, lsum = make_body(lambda u, t: None, last=True)(jnp.int32(NU - 1), carry)
    att = (att_s[...] + project(jnp.int32(NU - 1), acc, lsum))[0:B]

    x2 = x + ga * att
    h2 = (_ln(x2) * (1.0 + cb) + sb).astype(bf16)
    wait_all(w1_v, S_W1)
    hh = b1_v[...].astype(f32).reshape(1, F)
    for c, wc in enumerate(_cols(w1_v, 0, F // 8, CT)):
        hh = hh + lax.dot_general(h2[:, c * 128:(c + 1) * 128], wc, NT_DIMS, preferred_element_type=f32)
    hh = jax.nn.gelu(hh, approximate=True).astype(bf16)
    y = b2_v[...].astype(f32).reshape(1, D)
    for g in range(3):
        for i in range(7):
            if W2G[i] == g:
                wait_all(w2_v.at[pl.ds(W2B[i], W2B[i + 1] - W2B[i])], S_W2 + i)
        for r0, r1 in W2R[g]:
            y = y + _matmul_cols(hh[:, r0:r1], _cols(w2_v, r0 // 8 * CT, (r1 - r0) // 8, CT))
    out_v[...] = (x2 + gb * y).astype(bf16)
    co = cp(out_v, o_hbm, S_OUT)
    co.start()
    co.wait()


def _tiles(w):
    r, c = w.shape
    return w.reshape(r // 8, 8, c // 128, 128).transpose(0, 2, 1, 3).reshape(-1, 8, 128)


CFG = dict()


@jax.jit
def pallas_adaLN_cond__sliding_block_cached__dense_activation_gelu__decode_kernel(A_x, A_k_cache, A_v_cache, A_wq, A_wo, B_x, B_w1, B_b1, B_w2, B_b2, c, w_mod):
    out = pl.pallas_call(
        functools.partial(kernel, CFG),
        in_specs=[pl.BlockSpec(memory_space=pl.ANY)] * 11,
        out_specs=pl.BlockSpec(memory_space=pl.ANY),
        out_shape=jax.ShapeDtypeStruct((B, D), bf16),
        scratch_shapes=[
            pltpu.VMEM((B, D), bf16), pltpu.VMEM((B, D), bf16), pltpu.VMEM((F,), bf16), pltpu.VMEM((D,), bf16),
            pltpu.VMEM((N_WQ, 8, 128), bf16), pltpu.VMEM((N_WO, 8, 128), bf16), pltpu.VMEM((N_W1, 8, 128), bf16),
            pltpu.VMEM((N_W2, 8, 128), bf16), pltpu.VMEM((N_WM, 8, 128), bf16),
            pltpu.VMEM((2 * NSLOT, W // 2, 2, DH), bf16),
            pltpu.VMEM((H, 8, DH), f32), pltpu.VMEM((8, D), f32), pltpu.VMEM((2, NT, 8, 128), f32),
            pltpu.VMEM((B, D), bf16),
            pltpu.SemaphoreType.DMA((NSEM,)),
        ],
        compiler_params=pltpu.CompilerParams(vmem_limit_bytes=64 * 1024 * 1024, disable_bounds_checks=True,
                                             disable_semaphore_checks=True),
    )(A_x.reshape(B, D), c, B_b1, B_b2,
      A_k_cache.reshape(B * H, S // 2, 2, DH), A_v_cache.reshape(B * H, S // 2, 2, DH),
      _tiles(A_wq), _tiles(A_wo), _tiles(B_w1.T), _tiles(B_w2), _tiles(w_mod))
    return out.reshape(B, 1, D)
```

```python
import functools

import jax
import jax.numpy as jnp
from jax import lax
import jax.experimental.pallas as pl
import jax.experimental.pallas.tpu as pltpu

B, D, H, S, DH, F = 4, 640, 32, 8192, 128, 1728
W = min(4096, max(256, S // 4))
NT = W // 128
NU = B * H
NSLOT = 16
G = 4
EPS = 1e-5
LOG2E = 1.4426950408889634
bf16 = jnp.bfloat16
f32 = jnp.float32
NT_DIMS = (((1,), (1,)), ((), ()))

PT = 16
CT = D // 128
N_WQ, N_WO, N_WM, N_W1, N_W2 = D * H * DH // 1024, H * DH * D // 1024, D * 6 * D // 1024, F * D // 1024, F * D // 1024

S_X, S_C, S_B1, S_B2, S_WM, S_WQ, S_WO, S_OUT, S_W1, S_W2, S_K, S_V = 0, 1, 2, 3, 4, 5, 6, 7, 8, 9, 16, 32
NSEM = S_V + NSLOT


def _ln(x):
    m = jnp.mean(x, axis=-1, keepdims=True)
    xc = x - m
    v = jnp.mean(xc * xc, axis=-1, keepdims=True)
    return xc / jnp.sqrt(v + EPS)


def _cols(w_v, lo, nslab, ct):
    blk = w_v[pl.ds(lo, nslab * ct)].reshape(nslab, ct, 8, 128)
    return [blk[:, c].reshape(nslab * 8, 128) for c in range(ct)]


def _matmul_cols(a, cols):
    return jnp.concatenate([jnp.dot(a, wc, preferred_element_type=f32) for wc in cols], axis=1)


def kernel(cfg, x_hbm, c_hbm, b1_hbm, b2_hbm, k_hbm, v_hbm, wq_hbm, wo_hbm, w1_hbm, w2_hbm, wm_hbm,
           o_hbm,
           x_v, c_v, b1_v, b2_v, wq_v, wo_v, w1_v, w2_v, wm_v, kvbuf, q_s, att_s, s_s, out_v, spin_s, sem):
    L = cfg.get("L", 5)
    UA = cfg.get("ua", 6)
    SK1, SK2 = cfg.get("skip1", 0), cfg.get("skip2", 12)
    PH_KV, PH_WM, PH_W1, PH_W2 = cfg.get("ph", (62, 7, 13, 3))
    NPACED, SPIN = cfg.get("nd", 20), cfg.get("spin", 8)
    assert 2 <= L and L + G <= NSLOT

    def cp(src, dst, i):
        return pltpu.make_async_copy(src, dst, sem.at[i])

    def wait_all(buf, i):
        pltpu.make_async_copy(buf, buf, sem.at[i]).wait()

    def loop(lo, hi, f):
        def body(i, c):
            f(i)
            return c
        lax.fori_loop(lo, hi, body, 0)

    def wpiece(hbm, vm, s0):
        def start(lo, prio, n=PT, g=0):
            cp(hbm.at[pl.ds(lo, n)], vm.at[pl.ds(lo, n)], s0 + g).start(priority=prio)
        return start
    wq_p = wpiece(wq_hbm, wq_v, S_WQ)
    wo_p = wpiece(wo_hbm, wo_v, S_WO)
    wm_p = wpiece(wm_hbm, wm_v, S_WM)
    w1_p = wpiece(w1_hbm, w1_v, S_W1)
    w2_p = wpiece(w2_hbm, w2_v, S_W2)

    KVB = [0] + [PH_KV + 64 * i for i in range(NT - 1)] + [W // 2]

    def head_of(u):
        return ((u >> 2) & 1) * (H // 2) + (u >> 3)

    def kv_start(u, j):
        row = (u & (B - 1)) * H + head_of(u)
        slot = u & (NSLOT - 1)
        n = KVB[j + 1] - KVB[j]
        src = pl.ds((S - W) // 2 + KVB[j], n)
        dst = pl.ds(KVB[j], n)
        cp(k_hbm.at[row, src], kvbuf.at[NSLOT + slot, dst], S_K + slot).start(priority=0)
        cp(v_hbm.at[row, src], kvbuf.at[slot, dst], S_V + slot).start(priority=1)

    def skew(v, t):
        e = t % G
        return v + L + (G - 1 - e), e * (NT // G) + t // G

    def k_wait(u):
        slot = u & (NSLOT - 1)
        wait_all(kvbuf.at[NSLOT + slot], S_K + slot)

    def v_wait(u):
        slot = u & (NSLOT - 1)
        wait_all(kvbuf.at[slot], S_V + slot)

    kv32 = kvbuf.bitcast(jnp.uint32).at[:, :, 0]

    def kv_tile(slot, t):
        return pltpu.bitcast(kv32[slot, pl.ds(t * 64, 64), :], bf16)

    small = [cp(x_hbm, x_v, S_X), cp(c_hbm, c_v, S_C), cp(b1_hbm, b1_v, S_B1), cp(b2_hbm, b2_v, S_B2)]
    HQ = N_WQ // 2
    NM = (N_WM - PH_WM) // PT // 2
    M1 = PH_WM + (NM + 1) * PT
    assert N_WO == N_WQ and HQ % PT == 0 and 0 < N_WM - (M1 + NM * PT) <= PT and NM <= HQ // PT

    def pro2(i):
        wq_p(i * PT, 0)
        wq_p(HQ + i * PT, 1)
        wo_p(i * PT, 0)
        wo_p(HQ + i * PT, 1)

    def pro3(i):
        pro2(i)
        wm_p(PH_WM + i * PT, 0)
        wm_p(M1 + i * PT, 1)

    def pro3_paced(i, z):
        for start, lo0, lo1 in ((wq_p, 0, HQ), (wo_p, 0, HQ), (wm_p, PH_WM, M1)):
            start(lo0 + i * PT, 0)
            start(lo1 + i * PT, 1)
            z = lax.fori_loop(0, SPIN, lambda j, c: (c * 5 + j) & 1023, z)
        return z
    spin_s[0] = lax.fori_loop(0, NPACED, pro3_paced, jnp.int32(1))
    loop(NPACED, NM, pro3)
    for s in small:
        s.start(priority=0)
    wm_p(PH_WM + NM * PT, 0)
    wm_p(M1 + NM * PT, 1, N_WM - (M1 + NM * PT))
    wm_p(0, 0, PH_WM)
    loop(NM, HQ // PT, pro2)

    def kv_prologue(v):
        for t in range(NT):
            u, j = skew(v, t)
            pl.when(u >= 0)(functools.partial(kv_start, u, j))
    V0 = -(L + G - 1)
    VA = min(0, V0 + UA)
    loop(V0, VA, kv_prologue)

    for s in small:
        s.wait()
    wait_all(wm_v, S_WM)
    cvec = c_v[...].astype(f32)
    x = x_v[...].astype(f32)
    mod = _matmul_cols((cvec * jax.nn.sigmoid(cvec)).astype(bf16), _cols(wm_v, 0, D // 8, 6 * CT))
    sa, ca, ga, sb, cb, gb = [mod[:, i * D:(i + 1) * D] for i in range(6)]
    h1 = (_ln(x) * (1.0 + ca) + sa).astype(bf16)
    wait_all(wq_v, S_WQ)
    for h, wc in enumerate(_cols(wq_v, 0, D // 8, H)):
        q_s[h, 0:B, :] = jnp.dot(h1, wc, preferred_element_type=f32)
    q_s[:, B:8, :] = jnp.zeros((H, 8 - B, DH), f32)
    att_s[...] = jnp.zeros(att_s.shape, f32)
    if VA < 0:
        loop(VA, 0, kv_prologue)

    cexp = (DH ** -0.5) * LOG2E
    row = lax.broadcasted_iota(jnp.int32, (8, DH), 0)

    def qk_tile(qh, u, t):
        return lax.dot_general(qh, kv_tile(NSLOT + (u & (NSLOT - 1)), t), NT_DIMS, preferred_element_type=f32)

    def project(u, acc, lsum):
        l = jnp.sum(lsum, axis=-1, keepdims=True)
        o = jnp.where(row == (u & (B - 1)), acc / l, 0.0).astype(bf16)
        h = head_of(jnp.maximum(u, 0))
        return _matmul_cols(o, _cols(wo_v, h * (DH // 8 * CT), DH // 8, CT))

    def make_body(issue, last=False):
        def body(u, carry):
            mx, acc_p, lsum_p = carry
            par = u & 1
            m = jnp.max(mx, axis=-1, keepdims=True)
            if not last:
                k_wait(u + 1)
                qn = q_s[head_of(u + 1)].astype(bf16)
            v_wait(u)
            att_s[...] += project(u - 1, acc_p, lsum_p)
            mxn = lsum = acc = None
            for t in range(NT):
                if not last:
                    st = qk_tile(qn, u + 1, t)
                    s_s[1 - par, t] = st
                    mxn = st if mxn is None else jnp.maximum(mxn, st)
                p = jnp.exp2((s_s[par, t] - m) * cexp)
                lsum = p if lsum is None else lsum + p
                pv = jnp.dot(p.astype(bf16), kv_tile(u & (NSLOT - 1), t), preferred_element_type=f32)
                acc = pv if acc is None else acc + pv
                issue(u, t)
            return (mx if last else mxn), acc, lsum
        return body

    wait_all(wo_v, S_WO)
    k_wait(0)
    q0 = q_s[0].astype(bf16)
    mx = None
    for t in range(NT):
        st = qk_tile(q0, 0, t)
        s_s[0, t] = st
        mx = st if mx is None else jnp.maximum(mx, st)

    VM = NU - (L + G - 1)
    free = [(v, t) for v in range(VM, NU - 1) for t in range(NT) if skew(v, t)[0] >= NU]
    N1 = (N_W1 - PH_W1) // PT
    N2 = (N_W2 - PH_W2) // PT
    NS2, RB2 = cfg.get("ns2", 20), cfg.get("rb2", 15)
    assert SK1 + N1 <= len(free) and SK2 + N2 <= len(free) and N1 >= 64 and N2 >= 3 * NS2
    assert all((i * 43) >> 7 == i // 3 for i in range(N2))

    def slot_index(d, t, minimum, where):
        nfree = minimum(d + 1, G)
        before = where(d < G, d * (d + 1) // 2 * (NT // G), (G * (G - 1) // 2) * (NT // G) + (d - (G - 1)) * NT)
        return before + (t // G) * nfree + (t % G)
    for i, (v, t) in enumerate(free):
        assert slot_index(v - VM, t, min, lambda c, a, b: a if c else b) == i

    W2B = [0] + [PH_W2 + (s * NS2 + o) * PT for s in range(3) for o in (RB2, NS2)] + [N_W2]
    W2G = [0, 1, 0, 1, 0, 1, 2]
    W2R = [[], [], []]
    for r in range(0, F, 128):
        r1 = min(r + 128, F)
        g = max(W2G[i] for i in range(7) if W2B[i] < r1 // 8 * CT and W2B[i + 1] > r // 8 * CT)
        if W2R[g] and W2R[g][-1][1] == r:
            W2R[g][-1][1] = r1
        else:
            W2R[g].append([r, r1])

    def issue_main(v, t):
        kv_start(*skew(v, t))

    def issue_end(v, t):
        u, j = skew(v, t)
        pl.when(u < NU)(functools.partial(kv_start, u, j))
        idx = slot_index(v - VM, t, jnp.minimum, jnp.where)

        @pl.when(jnp.logical_and(u >= NU, jnp.logical_and(idx >= SK1, idx < SK1 + N1)))
        def _():
            i = idx - SK1
            w1_p(PH_W1 + jnp.where(i < 64, (i & 3) * 16 + (i >> 2), i) * PT, 0)

        @pl.when(jnp.logical_and(u >= NU, jnp.logical_and(idx >= SK2, idx < SK2 + N2)))
        def _():
            i = idx - SK2
            rnd = (i * 43) >> 7
            rr = i < 3 * NS2
            st = i - 3 * rnd
            w2_p(PH_W2 + jnp.where(rr, st * NS2 + rnd, i) * PT, 1,
                 g=jnp.where(rr, 2 * st + (rnd >= RB2).astype(jnp.int32), 6))

        @pl.when(jnp.logical_and(u >= NU, idx == SK2 + N2 - 1))
        def _():
            w2_p(PH_W2 + N2 * PT, 1, N_W2 - PH_W2 - N2 * PT, g=6)

    carry = (mx, jnp.zeros((8, DH), f32), jnp.ones((8, DH), f32))
    carry = lax.fori_loop(0, VM, make_body(issue_main), carry)
    w1_p(0, 0, PH_W1)
    w1_p(PH_W1 + N1 * PT, 0, N_W1 - PH_W1 - N1 * PT)
    w2_p(0, 1, PH_W2)
    carry = lax.fori_loop(VM, NU - 1, make_body(issue_end), carry)
    _, acc, lsum = make_body(lambda u, t: None, last=True)(jnp.int32(NU - 1), carry)
    att = (att_s[...] + project(jnp.int32(NU - 1), acc, lsum))[0:B]

    x2 = x + ga * att
    h2 = (_ln(x2) * (1.0 + cb) + sb).astype(bf16)
    wait_all(w1_v, S_W1)
    hh = b1_v[...].astype(f32).reshape(1, F)
    for c, wc in enumerate(_cols(w1_v, 0, F // 8, CT)):
        hh = hh + lax.dot_general(h2[:, c * 128:(c + 1) * 128], wc, NT_DIMS, preferred_element_type=f32)
    hh = jax.nn.gelu(hh, approximate=True).astype(bf16)
    y = b2_v[...].astype(f32).reshape(1, D)
    for g in range(3):
        for i in range(7):
            if W2G[i] == g:
                wait_all(w2_v.at[pl.ds(W2B[i], W2B[i + 1] - W2B[i])], S_W2 + i)
        for r0, r1 in W2R[g]:
            y = y + _matmul_cols(hh[:, r0:r1], _cols(w2_v, r0 // 8 * CT, (r1 - r0) // 8, CT))
    out_v[...] = (x2 + gb * y).astype(bf16)
    co = cp(out_v, o_hbm, S_OUT)
    co.start()
    co.wait()


def _tiles(w):
    r, c = w.shape
    return w.reshape(r // 8, 8, c // 128, 128).transpose(0, 2, 1, 3).reshape(-1, 8, 128)


CFG = dict()


@jax.jit
def pallas_adaLN_cond__sliding_block_cached__dense_activation_gelu__decode_kernel(A_x, A_k_cache, A_v_cache, A_wq, A_wo, B_x, B_w1, B_b1, B_w2, B_b2, c, w_mod):
    out = pl.pallas_call(
        functools.partial(kernel, CFG),
        in_specs=[pl.BlockSpec(memory_space=pl.ANY)] * 11,
        out_specs=pl.BlockSpec(memory_space=pl.ANY),
        out_shape=jax.ShapeDtypeStruct((B, D), bf16),
        scratch_shapes=[
            pltpu.VMEM((B, D), bf16), pltpu.VMEM((B, D), bf16), pltpu.VMEM((F,), bf16), pltpu.VMEM((D,), bf16),
            pltpu.VMEM((N_WQ, 8, 128), bf16), pltpu.VMEM((N_WO, 8, 128), bf16), pltpu.VMEM((N_W1, 8, 128), bf16),
            pltpu.VMEM((N_W2, 8, 128), bf16), pltpu.VMEM((N_WM, 8, 128), bf16),
            pltpu.VMEM((2 * NSLOT, W // 2, 2, DH), bf16),
            pltpu.VMEM((H, 8, DH), f32), pltpu.VMEM((8, D), f32), pltpu.VMEM((2, NT, 8, 128), f32),
            pltpu.VMEM((B, D), bf16), pltpu.SMEM((1,), jnp.int32),
            pltpu.SemaphoreType.DMA((NSEM,)),
        ],
        compiler_params=pltpu.CompilerParams(vmem_limit_bytes=64 * 1024 * 1024, disable_bounds_checks=True,
                                             disable_semaphore_checks=True),
    )(A_x.reshape(B, D), c, B_b1, B_b2,
      A_k_cache.reshape(B * H, S // 2, 2, DH), A_v_cache.reshape(B * H, S // 2, 2, DH),
      _tiles(A_wq), _tiles(A_wo), _tiles(B_w1.T), _tiles(B_w2), _tiles(w_mod))
    return out.reshape(B, 1, D)
```

```python
import functools

import jax
import jax.numpy as jnp
from jax import lax
import jax.experimental.pallas as pl
import jax.experimental.pallas.tpu as pltpu

B, D, H, S, DH, F = 4, 640, 32, 8192, 128, 1728
W = min(4096, max(256, S // 4))
NT = W // 128
NU = B * H
NSLOT = 16
G = 4
EPS = 1e-5
LOG2E = 1.4426950408889634
bf16 = jnp.bfloat16
f32 = jnp.float32
NT_DIMS = (((1,), (1,)), ((), ()))

PT = 16
CT = D // 128
N_WQ, N_WO, N_WM, N_W1, N_W2 = D * H * DH // 1024, H * DH * D // 1024, D * 6 * D // 1024, F * D // 1024, F * D // 1024

S_X, S_C, S_B1, S_B2, S_WM, S_WQ, S_WO, S_OUT, S_W1, S_W2, S_K, S_V = 0, 1, 2, 3, 4, 5, 6, 7, 8, 9, 16, 32
NSEM = S_V + NSLOT


def _ln(x):
    m = jnp.mean(x, axis=-1, keepdims=True)
    xc = x - m
    v = jnp.mean(xc * xc, axis=-1, keepdims=True)
    return xc / jnp.sqrt(v + EPS)


def _cols(w_v, lo, nslab, ct):
    blk = w_v[pl.ds(lo, nslab * ct)].reshape(nslab, ct, 8, 128)
    return [blk[:, c].reshape(nslab * 8, 128) for c in range(ct)]


def _matmul_cols(a, cols):
    return jnp.concatenate([jnp.dot(a, wc, preferred_element_type=f32) for wc in cols], axis=1)


def kernel(cfg, x_hbm, c_hbm, b1_hbm, b2_hbm, k_hbm, v_hbm, wq_hbm, wo_hbm, w1_hbm, w2_hbm, wm_hbm,
           o_hbm,
           x_v, c_v, b1_v, b2_v, wq_v, wo_v, w1_v, w2_v, wm_v, kvbuf, q_s, att_s, s_s, out_v, spin_s, sem):
    L = cfg.get("L", 5)
    UA = cfg.get("ua", 6)
    SK1, SK2 = cfg.get("skip1", 0), cfg.get("skip2", 16)
    PH_KV, PH_WM, PH_W1, PH_W2 = cfg.get("ph", (31, 7, 13, 3))
    NPACED, SPIN = cfg.get("nd", 20), cfg.get("spin", 8)
    assert 2 <= L and L + G <= NSLOT

    def cp(src, dst, i):
        return pltpu.make_async_copy(src, dst, sem.at[i])

    def wait_all(buf, i):
        pltpu.make_async_copy(buf, buf, sem.at[i]).wait()

    def loop(lo, hi, f):
        def body(i, c):
            f(i)
            return c
        lax.fori_loop(lo, hi, body, 0)

    def wpiece(hbm, vm, s0):
        def start(lo, prio, n=PT, g=0):
            cp(hbm.at[pl.ds(lo, n)], vm.at[pl.ds(lo, n)], s0 + g).start(priority=prio)
        return start
    wq_p = wpiece(wq_hbm, wq_v, S_WQ)
    wo_p = wpiece(wo_hbm, wo_v, S_WO)
    wm_p = wpiece(wm_hbm, wm_v, S_WM)
    w1_p = wpiece(w1_hbm, w1_v, S_W1)
    w2_p = wpiece(w2_hbm, w2_v, S_W2)

    KVB = [0] + [PH_KV + 32 * i for i in range(NT - 1)] + [W // 4]

    def head_of(u):
        return ((u >> 2) & 1) * (H // 2) + (u >> 3)

    def kv_start(u, j):
        row = (u & (B - 1)) * H + head_of(u)
        slot = u & (NSLOT - 1)
        n = KVB[j + 1] - KVB[j]
        src = pl.ds((S - W) // 4 + KVB[j], n)
        dst = pl.ds(KVB[j], n)
        cp(k_hbm.at[row, src], kvbuf.at[NSLOT + slot, dst], S_K + slot).start(priority=0)
        cp(v_hbm.at[row, src], kvbuf.at[slot, dst], S_V + slot).start(priority=1)

    def skew(v, t):
        e = t % G
        return v + L + (G - 1 - e), e * (NT // G) + t // G

    def k_wait(u):
        slot = u & (NSLOT - 1)
        wait_all(kvbuf.at[NSLOT + slot], S_K + slot)

    def v_wait(u):
        slot = u & (NSLOT - 1)
        wait_all(kvbuf.at[slot], S_V + slot)

    def kv_tile(slot, t):
        w = pltpu.bitcast(kvbuf[slot, pl.ds(t * 32, 32)], jnp.uint32)
        return pltpu.bitcast(jnp.concatenate([w[i] for i in range(32)], axis=0), bf16)

    small = [cp(x_hbm, x_v, S_X), cp(c_hbm, c_v, S_C), cp(b1_hbm, b1_v, S_B1), cp(b2_hbm, b2_v, S_B2)]
    HQ = N_WQ // 2
    NM = (N_WM - PH_WM) // PT // 2
    M1 = PH_WM + (NM + 1) * PT
    assert N_WO == N_WQ and HQ % PT == 0 and 0 < N_WM - (M1 + NM * PT) <= PT and NM <= HQ // PT

    def pro2(i):
        wq_p(i * PT, 0)
        wq_p(HQ + i * PT, 1)
        wo_p(i * PT, 0)
        wo_p(HQ + i * PT, 1)

    def pro3(i):
        pro2(i)
        wm_p(PH_WM + i * PT, 0)
        wm_p(M1 + i * PT, 1)

    def pro3_paced(i, z):
        for start, lo0, lo1 in ((wq_p, 0, HQ), (wo_p, 0, HQ), (wm_p, PH_WM, M1)):
            start(lo0 + i * PT, 0)
            start(lo1 + i * PT, 1)
            z = lax.fori_loop(0, SPIN, lambda j, c: (c * 5 + j) & 1023, z)
        return z
    spin_s[0] = lax.fori_loop(0, NPACED, pro3_paced, jnp.int32(1))
    loop(NPACED, NM, pro3)
    for s in small:
        s.start(priority=0)
    wm_p(PH_WM + NM * PT, 0)
    wm_p(M1 + NM * PT, 1, N_WM - (M1 + NM * PT))
    wm_p(0, 0, PH_WM)
    loop(NM, HQ // PT, pro2)

    def kv_prologue(v):
        for t in range(NT):
            u, j = skew(v, t)
            pl.when(u >= 0)(functools.partial(kv_start, u, j))
    V0 = -(L + G - 1)
    VA = min(0, V0 + UA)
    loop(V0, VA, kv_prologue)

    for s in small:
        s.wait()
    wait_all(wm_v, S_WM)
    cvec = c_v[...].astype(f32)
    x = x_v[...].astype(f32)
    mod = _matmul_cols((cvec * jax.nn.sigmoid(cvec)).astype(bf16), _cols(wm_v, 0, D // 8, 6 * CT))
    sa, ca, ga, sb, cb, gb = [mod[:, i * D:(i + 1) * D] for i in range(6)]
    h1 = (_ln(x) * (1.0 + ca) + sa).astype(bf16)
    wait_all(wq_v, S_WQ)
    for h, wc in enumerate(_cols(wq_v, 0, D // 8, H)):
        q_s[h, 0:B, :] = jnp.dot(h1, wc, preferred_element_type=f32)
    q_s[:, B:8, :] = jnp.zeros((H, 8 - B, DH), f32)
    att_s[...] = jnp.zeros(att_s.shape, f32)
    if VA < 0:
        loop(VA, 0, kv_prologue)

    cexp = (DH ** -0.5) * LOG2E
    row = lax.broadcasted_iota(jnp.int32, (8, DH), 0)

    def qk_tile(qh, u, t):
        return lax.dot_general(qh, kv_tile(NSLOT + (u & (NSLOT - 1)), t), NT_DIMS, preferred_element_type=f32)

    def project(u, acc, lsum):
        l = jnp.sum(lsum, axis=-1, keepdims=True)
        o = jnp.where(row == (u & (B - 1)), acc / l, 0.0).astype(bf16)
        h = head_of(jnp.maximum(u, 0))
        return _matmul_cols(o, _cols(wo_v, h * (DH // 8 * CT), DH // 8, CT))

    def make_body(issue, last=False):
        def body(u, carry):
            mx, acc_p, lsum_p = carry
            par = u & 1
            m = jnp.max(mx, axis=-1, keepdims=True)
            if not last:
                k_wait(u + 1)
                qn = q_s[head_of(u + 1)].astype(bf16)
            v_wait(u)
            att_s[...] += project(u - 1, acc_p, lsum_p)
            mxn = lsum = acc = None
            for t in range(NT):
                if not last:
                    st = qk_tile(qn, u + 1, t)
                    s_s[1 - par, t] = st
                    mxn = st if mxn is None else jnp.maximum(mxn, st)
                p = jnp.exp2((s_s[par, t] - m) * cexp)
                lsum = p if lsum is None else lsum + p
                pv = jnp.dot(p.astype(bf16), kv_tile(u & (NSLOT - 1), t), preferred_element_type=f32)
                acc = pv if acc is None else acc + pv
                issue(u, t)
            return (mx if last else mxn), acc, lsum
        return body

    wait_all(wo_v, S_WO)
    k_wait(0)
    q0 = q_s[0].astype(bf16)
    mx = None
    for t in range(NT):
        st = qk_tile(q0, 0, t)
        s_s[0, t] = st
        mx = st if mx is None else jnp.maximum(mx, st)

    VM = NU - (L + G - 1)
    free = [(v, t) for v in range(VM, NU - 1) for t in range(NT) if skew(v, t)[0] >= NU]
    N1 = (N_W1 - PH_W1) // PT
    N2 = (N_W2 - PH_W2) // PT
    NS2, RB2 = cfg.get("ns2", 20), cfg.get("rb2", 15)
    assert SK1 + N1 <= len(free) and SK2 + N2 <= len(free) and N1 >= 64 and N2 >= 3 * NS2
    assert all((i * 43) >> 7 == i // 3 for i in range(N2))

    def slot_index(d, t, minimum, where):
        nfree = minimum(d + 1, G)
        before = where(d < G, d * (d + 1) // 2 * (NT // G), (G * (G - 1) // 2) * (NT // G) + (d - (G - 1)) * NT)
        return before + (t // G) * nfree + (t % G)
    for i, (v, t) in enumerate(free):
        assert slot_index(v - VM, t, min, lambda c, a, b: a if c else b) == i

    W2B = [0] + [PH_W2 + (s * NS2 + o) * PT for s in range(3) for o in (RB2, NS2)] + [N_W2]
    W2G = [0, 1, 0, 1, 0, 1, 2]
    W2R = [[], [], []]
    for r in range(0, F, 128):
        r1 = min(r + 128, F)
        g = max(W2G[i] for i in range(7) if W2B[i] < r1 // 8 * CT and W2B[i + 1] > r // 8 * CT)
        if W2R[g] and W2R[g][-1][1] == r:
            W2R[g][-1][1] = r1
        else:
            W2R[g].append([r, r1])

    def issue_main(v, t):
        kv_start(*skew(v, t))

    def issue_end(v, t):
        u, j = skew(v, t)
        pl.when(u < NU)(functools.partial(kv_start, u, j))
        idx = slot_index(v - VM, t, jnp.minimum, jnp.where)

        @pl.when(jnp.logical_and(u >= NU, jnp.logical_and(idx >= SK1, idx < SK1 + N1)))
        def _():
            i = idx - SK1
            w1_p(PH_W1 + jnp.where(i < 64, (i & 3) * 16 + (i >> 2), i) * PT, 0)

        @pl.when(jnp.logical_and(u >= NU, jnp.logical_and(idx >= SK2, idx < SK2 + N2)))
        def _():
            i = idx - SK2
            rnd = (i * 43) >> 7
            rr = i < 3 * NS2
            st = i - 3 * rnd
            w2_p(PH_W2 + jnp.where(rr, st * NS2 + rnd, i) * PT, 1,
                 g=jnp.where(rr, 2 * st + (rnd >= RB2).astype(jnp.int32), 6))

        @pl.when(jnp.logical_and(u >= NU, idx == SK2 + N2 - 1))
        def _():
            w2_p(PH_W2 + N2 * PT, 1, N_W2 - PH_W2 - N2 * PT, g=6)

    carry = (mx, jnp.zeros((8, DH), f32), jnp.ones((8, DH), f32))
    carry = lax.fori_loop(0, VM, make_body(issue_main), carry)
    w1_p(0, 0, PH_W1)
    w1_p(PH_W1 + N1 * PT, 0, N_W1 - PH_W1 - N1 * PT)
    w2_p(0, 1, PH_W2)
    carry = lax.fori_loop(VM, NU - 1, make_body(issue_end), carry)
    _, acc, lsum = make_body(lambda u, t: None, last=True)(jnp.int32(NU - 1), carry)
    att = (att_s[...] + project(jnp.int32(NU - 1), acc, lsum))[0:B]

    x2 = x + ga * att
    h2 = (_ln(x2) * (1.0 + cb) + sb).astype(bf16)
    wait_all(w1_v, S_W1)
    hh = b1_v[...].astype(f32).reshape(1, F)
    for c, wc in enumerate(_cols(w1_v, 0, F // 8, CT)):
        hh = hh + lax.dot_general(h2[:, c * 128:(c + 1) * 128], wc, NT_DIMS, preferred_element_type=f32)
    hh = jax.nn.gelu(hh, approximate=True).astype(bf16)
    y = b2_v[...].astype(f32).reshape(1, D)
    for g in range(3):
        for i in range(7):
            if W2G[i] == g:
                wait_all(w2_v.at[pl.ds(W2B[i], W2B[i + 1] - W2B[i])], S_W2 + i)
        for r0, r1 in W2R[g]:
            y = y + _matmul_cols(hh[:, r0:r1], _cols(w2_v, r0 // 8 * CT, (r1 - r0) // 8, CT))
    out_v[...] = (x2 + gb * y).astype(bf16)
    co = cp(out_v, o_hbm, S_OUT)
    co.start()
    co.wait()


def _tiles(w):
    r, c = w.shape
    return w.reshape(r // 8, 8, c // 128, 128).transpose(0, 2, 1, 3).reshape(-1, 8, 128)


CFG = dict()


@jax.jit
def pallas_adaLN_cond__sliding_block_cached__dense_activation_gelu__decode_kernel(A_x, A_k_cache, A_v_cache, A_wq, A_wo, B_x, B_w1, B_b1, B_w2, B_b2, c, w_mod):
    out = pl.pallas_call(
        functools.partial(kernel, CFG),
        in_specs=[pl.BlockSpec(memory_space=pl.ANY)] * 11,
        out_specs=pl.BlockSpec(memory_space=pl.ANY),
        out_shape=jax.ShapeDtypeStruct((B, D), bf16),
        scratch_shapes=[
            pltpu.VMEM((B, D), bf16), pltpu.VMEM((B, D), bf16), pltpu.VMEM((F,), bf16), pltpu.VMEM((D,), bf16),
            pltpu.VMEM((N_WQ, 8, 128), bf16), pltpu.VMEM((N_WO, 8, 128), bf16), pltpu.VMEM((N_W1, 8, 128), bf16),
            pltpu.VMEM((N_W2, 8, 128), bf16), pltpu.VMEM((N_WM, 8, 128), bf16),
            pltpu.VMEM((2 * NSLOT, W // 4, 4, DH), bf16),
            pltpu.VMEM((H, 8, DH), f32), pltpu.VMEM((8, D), f32), pltpu.VMEM((2, NT, 8, 128), f32),
            pltpu.VMEM((B, D), bf16), pltpu.SMEM((1,), jnp.int32),
            pltpu.SemaphoreType.DMA((NSEM,)),
        ],
        compiler_params=pltpu.CompilerParams(vmem_limit_bytes=64 * 1024 * 1024, disable_bounds_checks=True,
                                             disable_semaphore_checks=True),
    )(A_x.reshape(B, D), c, B_b1, B_b2,
      A_k_cache.reshape(B * H, S // 4, 4, DH), A_v_cache.reshape(B * H, S // 4, 4, DH),
      _tiles(A_wq), _tiles(A_wo), _tiles(B_w1.T), _tiles(B_w2), _tiles(w_mod))
    return out.reshape(B, 1, D)
```

```python
import functools

import jax
import jax.numpy as jnp
from jax import lax
import jax.experimental.pallas as pl
import jax.experimental.pallas.tpu as pltpu

B, D, H, S, DH, F = 4, 640, 32, 8192, 128, 1728
W = min(4096, max(256, S // 4))
NT = W // 128
NU = B * H
NSLOT = 16
G = 4
EPS = 1e-5
LOG2E = 1.4426950408889634
bf16 = jnp.bfloat16
f32 = jnp.float32
NT_DIMS = (((1,), (1,)), ((), ()))

PT = 16
CT = D // 128
N_WQ, N_WO, N_WM, N_W1, N_W2 = D * H * DH // 1024, H * DH * D // 1024, D * 6 * D // 1024, F * D // 1024, F * D // 1024

L = 5
UA = 6
NPACED, SPIN = 20, 8
SK1, SK2 = 0, 16
NS2, RB2 = 20, 15
PH_KV, PH_WM, PH_W1, PH_W2 = 31, 7, 13, 3

S_X, S_C, S_B1, S_B2, S_WM, S_WQ, S_WO, S_OUT, S_W1, S_W2, S_K, S_V = 0, 1, 2, 3, 4, 5, 6, 7, 8, 9, 16, 32
NSEM = S_V + NSLOT


def _ln(x):
    m = jnp.mean(x, axis=-1, keepdims=True)
    xc = x - m
    v = jnp.mean(xc * xc, axis=-1, keepdims=True)
    return xc / jnp.sqrt(v + EPS)


def _cols(w_v, lo, nslab, ct):
    blk = w_v[pl.ds(lo, nslab * ct)].reshape(nslab, ct, 8, 128)
    return [blk[:, c].reshape(nslab * 8, 128) for c in range(ct)]


def _matmul_cols(a, cols):
    return jnp.concatenate([jnp.dot(a, wc, preferred_element_type=f32) for wc in cols], axis=1)


def _kernel(x_hbm, c_hbm, b1_hbm, b2_hbm, k_hbm, v_hbm, wq_hbm, wo_hbm, w1_hbm, w2_hbm, wm_hbm,
            o_hbm,
            x_v, c_v, b1_v, b2_v, wq_v, wo_v, w1_v, w2_v, wm_v, kvbuf, q_s, att_s, s_s, out_v, spin_s, sem):
    assert 2 <= L and L + G <= NSLOT

    def cp(src, dst, i):
        return pltpu.make_async_copy(src, dst, sem.at[i])

    def wait_all(buf, i):
        pltpu.make_async_copy(buf, buf, sem.at[i]).wait()

    def loop(lo, hi, f):
        def body(i, c):
            f(i)
            return c
        lax.fori_loop(lo, hi, body, 0)

    def wpiece(hbm, vm, s0):
        def start(lo, prio, n=PT, g=0):
            cp(hbm.at[pl.ds(lo, n)], vm.at[pl.ds(lo, n)], s0 + g).start(priority=prio)
        return start
    wq_p = wpiece(wq_hbm, wq_v, S_WQ)
    wo_p = wpiece(wo_hbm, wo_v, S_WO)
    wm_p = wpiece(wm_hbm, wm_v, S_WM)
    w1_p = wpiece(w1_hbm, w1_v, S_W1)
    w2_p = wpiece(w2_hbm, w2_v, S_W2)

    KVB = [0] + [PH_KV + 32 * i for i in range(NT - 1)] + [W // 4]

    def head_of(u):
        return ((u >> 2) & 1) * (H // 2) + (u >> 3)

    def kv_start(u, j):
        row = (u & (B - 1)) * H + head_of(u)
        slot = u & (NSLOT - 1)
        n = KVB[j + 1] - KVB[j]
        src = pl.ds((S - W) // 4 + KVB[j], n)
        dst = pl.ds(KVB[j], n)
        cp(k_hbm.at[row, src], kvbuf.at[NSLOT + slot, dst], S_K + slot).start(priority=0)
        cp(v_hbm.at[row, src], kvbuf.at[slot, dst], S_V + slot).start(priority=1)

    def skew(v, t):
        e = t % G
        return v + L + (G - 1 - e), e * (NT // G) + t // G

    def k_wait(u):
        slot = u & (NSLOT - 1)
        wait_all(kvbuf.at[NSLOT + slot], S_K + slot)

    def v_wait(u):
        slot = u & (NSLOT - 1)
        wait_all(kvbuf.at[slot], S_V + slot)

    def kv_tile(slot, t):
        w = pltpu.bitcast(kvbuf[slot, pl.ds(t * 32, 32)], jnp.uint32)
        return pltpu.bitcast(jnp.concatenate([w[i] for i in range(32)], axis=0), bf16)

    small = [cp(x_hbm, x_v, S_X), cp(c_hbm, c_v, S_C), cp(b1_hbm, b1_v, S_B1), cp(b2_hbm, b2_v, S_B2)]
    HQ = N_WQ // 2
    NM = (N_WM - PH_WM) // PT // 2
    M1 = PH_WM + (NM + 1) * PT
    assert N_WO == N_WQ and HQ % PT == 0 and 0 < N_WM - (M1 + NM * PT) <= PT and NM <= HQ // PT

    def pro2(i):
        wq_p(i * PT, 0)
        wq_p(HQ + i * PT, 1)
        wo_p(i * PT, 0)
        wo_p(HQ + i * PT, 1)

    def pro3(i):
        pro2(i)
        wm_p(PH_WM + i * PT, 0)
        wm_p(M1 + i * PT, 1)

    def pro3_paced(i, z):
        for start, lo0, lo1 in ((wq_p, 0, HQ), (wo_p, 0, HQ), (wm_p, PH_WM, M1)):
            start(lo0 + i * PT, 0)
            start(lo1 + i * PT, 1)
            z = lax.fori_loop(0, SPIN, lambda j, c: (c * 5 + j) & 1023, z)
        return z
    spin_s[0] = lax.fori_loop(0, NPACED, pro3_paced, jnp.int32(1))
    loop(NPACED, NM, pro3)
    for s in small:
        s.start(priority=0)
    wm_p(PH_WM + NM * PT, 0)
    wm_p(M1 + NM * PT, 1, N_WM - (M1 + NM * PT))
    wm_p(0, 0, PH_WM)
    loop(NM, HQ // PT, pro2)

    def kv_prologue(v):
        for t in range(NT):
            u, j = skew(v, t)
            pl.when(u >= 0)(functools.partial(kv_start, u, j))
    V0 = -(L + G - 1)
    VA = min(0, V0 + UA)
    loop(V0, VA, kv_prologue)

    for s in small:
        s.wait()
    wait_all(wm_v, S_WM)
    cvec = c_v[...].astype(f32)
    x = x_v[...].astype(f32)
    mod = _matmul_cols((cvec * jax.nn.sigmoid(cvec)).astype(bf16), _cols(wm_v, 0, D // 8, 6 * CT))
    sa, ca, ga, sb, cb, gb = [mod[:, i * D:(i + 1) * D] for i in range(6)]
    h1 = (_ln(x) * (1.0 + ca) + sa).astype(bf16)
    wait_all(wq_v, S_WQ)
    for h, wc in enumerate(_cols(wq_v, 0, D // 8, H)):
        q_s[h, 0:B, :] = jnp.dot(h1, wc, preferred_element_type=f32)
    q_s[:, B:8, :] = jnp.zeros((H, 8 - B, DH), f32)
    att_s[...] = jnp.zeros(att_s.shape, f32)
    if VA < 0:
        loop(VA, 0, kv_prologue)

    cexp = (DH ** -0.5) * LOG2E
    row = lax.broadcasted_iota(jnp.int32, (8, DH), 0)

    def qk_tile(qh, u, t):
        return lax.dot_general(qh, kv_tile(NSLOT + (u & (NSLOT - 1)), t), NT_DIMS, preferred_element_type=f32)

    def project(u, acc, lsum):
        l = jnp.sum(lsum, axis=-1, keepdims=True)
        o = jnp.where(row == (u & (B - 1)), acc / l, 0.0).astype(bf16)
        h = head_of(jnp.maximum(u, 0))
        return _matmul_cols(o, _cols(wo_v, h * (DH // 8 * CT), DH // 8, CT))

    def make_body(issue, last=False):
        def body(u, carry):
            mx, acc_p, lsum_p = carry
            par = u & 1
            m = jnp.max(mx, axis=-1, keepdims=True)
            if not last:
                k_wait(u + 1)
                qn = q_s[head_of(u + 1)].astype(bf16)
            v_wait(u)
            att_s[...] += project(u - 1, acc_p, lsum_p)
            mxn = lsum = acc = None
            for t in range(NT):
                if not last:
                    st = qk_tile(qn, u + 1, t)
                    s_s[1 - par, t] = st
                    mxn = st if mxn is None else jnp.maximum(mxn, st)
                p = jnp.exp2((s_s[par, t] - m) * cexp)
                lsum = p if lsum is None else lsum + p
                pv = jnp.dot(p.astype(bf16), kv_tile(u & (NSLOT - 1), t), preferred_element_type=f32)
                acc = pv if acc is None else acc + pv
                issue(u, t)
            return (mx if last else mxn), acc, lsum
        return body

    wait_all(wo_v, S_WO)
    k_wait(0)
    q0 = q_s[0].astype(bf16)
    mx = None
    for t in range(NT):
        st = qk_tile(q0, 0, t)
        s_s[0, t] = st
        mx = st if mx is None else jnp.maximum(mx, st)

    VM = NU - (L + G - 1)
    free = [(v, t) for v in range(VM, NU - 1) for t in range(NT) if skew(v, t)[0] >= NU]
    N1 = (N_W1 - PH_W1) // PT
    N2 = (N_W2 - PH_W2) // PT
    assert SK1 + N1 <= len(free) and SK2 + N2 <= len(free) and N1 >= 64 and N2 >= 3 * NS2
    assert all((i * 43) >> 7 == i // 3 for i in range(N2))

    def slot_index(d, t, minimum, where):
        nfree = minimum(d + 1, G)
        before = where(d < G, d * (d + 1) // 2 * (NT // G), (G * (G - 1) // 2) * (NT // G) + (d - (G - 1)) * NT)
        return before + (t // G) * nfree + (t % G)
    for i, (v, t) in enumerate(free):
        assert slot_index(v - VM, t, min, lambda c, a, b: a if c else b) == i

    W2B = [0] + [PH_W2 + (s * NS2 + o) * PT for s in range(3) for o in (RB2, NS2)] + [N_W2]
    W2G = [0, 1, 0, 1, 0, 1, 2]
    W2R = [[], [], []]
    for r in range(0, F, 128):
        r1 = min(r + 128, F)
        g = max(W2G[i] for i in range(7) if W2B[i] < r1 // 8 * CT and W2B[i + 1] > r // 8 * CT)
        if W2R[g] and W2R[g][-1][1] == r:
            W2R[g][-1][1] = r1
        else:
            W2R[g].append([r, r1])

    def issue_main(v, t):
        kv_start(*skew(v, t))

    def issue_end(v, t):
        u, j = skew(v, t)
        pl.when(u < NU)(functools.partial(kv_start, u, j))
        idx = slot_index(v - VM, t, jnp.minimum, jnp.where)

        @pl.when(jnp.logical_and(u >= NU, jnp.logical_and(idx >= SK1, idx < SK1 + N1)))
        def _():
            i = idx - SK1
            w1_p(PH_W1 + jnp.where(i < 64, (i & 3) * 16 + (i >> 2), i) * PT, 0)

        @pl.when(jnp.logical_and(u >= NU, jnp.logical_and(idx >= SK2, idx < SK2 + N2)))
        def _():
            i = idx - SK2
            rnd = (i * 43) >> 7
            rr = i < 3 * NS2
            st = i - 3 * rnd
            w2_p(PH_W2 + jnp.where(rr, st * NS2 + rnd, i) * PT, 1,
                 g=jnp.where(rr, 2 * st + (rnd >= RB2).astype(jnp.int32), 6))

        @pl.when(jnp.logical_and(u >= NU, idx == SK2 + N2 - 1))
        def _():
            w2_p(PH_W2 + N2 * PT, 1, N_W2 - PH_W2 - N2 * PT, g=6)

    carry = (mx, jnp.zeros((8, DH), f32), jnp.ones((8, DH), f32))
    carry = lax.fori_loop(0, VM, make_body(issue_main), carry)
    w1_p(0, 0, PH_W1)
    w1_p(PH_W1 + N1 * PT, 0, N_W1 - PH_W1 - N1 * PT)
    w2_p(0, 1, PH_W2)
    carry = lax.fori_loop(VM, NU - 1, make_body(issue_end), carry)
    _, acc, lsum = make_body(lambda u, t: None, last=True)(jnp.int32(NU - 1), carry)
    att = (att_s[...] + project(jnp.int32(NU - 1), acc, lsum))[0:B]

    x2 = x + ga * att
    h2 = (_ln(x2) * (1.0 + cb) + sb).astype(bf16)
    wait_all(w1_v, S_W1)
    hh = b1_v[...].astype(f32).reshape(1, F)
    for c, wc in enumerate(_cols(w1_v, 0, F // 8, CT)):
        hh = hh + lax.dot_general(h2[:, c * 128:(c + 1) * 128], wc, NT_DIMS, preferred_element_type=f32)
    hh = jax.nn.gelu(hh, approximate=True).astype(bf16)
    y = b2_v[...].astype(f32).reshape(1, D)
    for g in range(3):
        for i in range(7):
            if W2G[i] == g:
                wait_all(w2_v.at[pl.ds(W2B[i], W2B[i + 1] - W2B[i])], S_W2 + i)
        for r0, r1 in W2R[g]:
            y = y + _matmul_cols(hh[:, r0:r1], _cols(w2_v, r0 // 8 * CT, (r1 - r0) // 8, CT))
    out_v[...] = (x2 + gb * y).astype(bf16)
    co = cp(out_v, o_hbm, S_OUT)
    co.start()
    co.wait()


def _tiles(w):
    r, c = w.shape
    return w.reshape(r // 8, 8, c // 128, 128).transpose(0, 2, 1, 3).reshape(-1, 8, 128)


@jax.jit
def pallas_adaLN_cond__sliding_block_cached__dense_activation_gelu__decode_kernel(A_x, A_k_cache, A_v_cache, A_wq, A_wo, B_x, B_w1, B_b1, B_w2, B_b2, c, w_mod):
    out = pl.pallas_call(
        _kernel,
        in_specs=[pl.BlockSpec(memory_space=pl.ANY)] * 11,
        out_specs=pl.BlockSpec(memory_space=pl.ANY),
        out_shape=jax.ShapeDtypeStruct((B, D), bf16),
        scratch_shapes=[
            pltpu.VMEM((B, D), bf16), pltpu.VMEM((B, D), bf16), pltpu.VMEM((F,), bf16), pltpu.VMEM((D,), bf16),
            pltpu.VMEM((N_WQ, 8, 128), bf16), pltpu.VMEM((N_WO, 8, 128), bf16), pltpu.VMEM((N_W1, 8, 128), bf16),
            pltpu.VMEM((N_W2, 8, 128), bf16), pltpu.VMEM((N_WM, 8, 128), bf16),
            pltpu.VMEM((2 * NSLOT, W // 4, 4, DH), bf16),
            pltpu.VMEM((H, 8, DH), f32), pltpu.VMEM((8, D), f32), pltpu.VMEM((2, NT, 8, 128), f32),
            pltpu.VMEM((B, D), bf16), pltpu.SMEM((1,), jnp.int32),
            pltpu.SemaphoreType.DMA((NSEM,)),
        ],
        compiler_params=pltpu.CompilerParams(vmem_limit_bytes=64 * 1024 * 1024, disable_bounds_checks=True,
                                             disable_semaphore_checks=True),
    )(A_x.reshape(B, D), c, B_b1, B_b2,
      A_k_cache.reshape(B * H, S // 4, 4, DH), A_v_cache.reshape(B * H, S // 4, 4, DH),
      _tiles(A_wq), _tiles(A_wo), _tiles(B_w1.T), _tiles(B_w2), _tiles(w_mod))
    return out.reshape(B, 1, D)
```

```python
import functools

import jax
import jax.numpy as jnp
from jax import lax
import jax.experimental.pallas as pl
import jax.experimental.pallas.tpu as pltpu

B, D, H, S, DH, F = 4, 640, 32, 8192, 128, 1728
W = min(4096, max(256, S // 4))
NT = W // 128
NU = B * H
NSLOT = 16
G = 4
EPS = 1e-5
LOG2E = 1.4426950408889634
bf16 = jnp.bfloat16
f32 = jnp.float32
NT_DIMS = (((1,), (1,)), ((), ()))

PT = 16
CT = D // 128
N_WQ, N_WO, N_WM, N_W1, N_W2 = D * H * DH // 1024, H * DH * D // 1024, D * 6 * D // 1024, F * D // 1024, F * D // 1024

L = 5
UA = 6
NPACED, SPIN = 20, 8
SK1, SK2 = 0, 16
NS2, RB2 = 20, 15
PH_KV, PH_WM, PH_W1, PH_W2 = 31, 7, 13, 3

S_X, S_C, S_B1, S_B2, S_WM, S_WQ, S_WO, S_OUT, S_W1, S_W2, S_K, S_V = 0, 1, 2, 3, 4, 5, 6, 7, 8, 9, 16, 32
NSEM = S_V + NSLOT


def _ln(x):
    m = jnp.mean(x, axis=-1, keepdims=True)
    xc = x - m
    v = jnp.mean(xc * xc, axis=-1, keepdims=True)
    return xc / jnp.sqrt(v + EPS)


def _cols(w_v, lo, nslab, ct):
    blk = w_v[pl.ds(lo, nslab * ct)].reshape(nslab, ct, 8, 128)
    return [blk[:, c].reshape(nslab * 8, 128) for c in range(ct)]


def _matmul_cols(a, cols):
    return jnp.concatenate([jnp.dot(a, wc, preferred_element_type=f32) for wc in cols], axis=1)


def _kernel(x_hbm, c_hbm, b1_hbm, b2_hbm, k_hbm, v_hbm, wq_hbm, wo_hbm, w1_hbm, w2_hbm, wm_hbm,
            o_hbm,
            x_v, c_v, b1_v, b2_v, wq_v, wo_v, w1_v, w2_v, wm_v, kvbuf, q_s, att_s, s_s, out_v, spin_s, sem):
    assert 2 <= L and L + G <= NSLOT

    def cp(src, dst, i):
        return pltpu.make_async_copy(src, dst, sem.at[i])

    def wait_all(buf, i):
        pltpu.make_async_copy(buf, buf, sem.at[i]).wait()

    def loop(lo, hi, f):
        def body(i, c):
            f(i)
            return c
        lax.fori_loop(lo, hi, body, 0)

    def wpiece(hbm, vm, s0):
        def start(lo, prio, n=PT, g=0):
            cp(hbm.at[pl.ds(lo, n)], vm.at[pl.ds(lo, n)], s0 + g).start(priority=prio)
        return start
    wq_p = wpiece(wq_hbm, wq_v, S_WQ)
    wo_p = wpiece(wo_hbm, wo_v, S_WO)
    wm_p = wpiece(wm_hbm, wm_v, S_WM)
    w1_p = wpiece(w1_hbm, w1_v, S_W1)
    w2_p = wpiece(w2_hbm, w2_v, S_W2)

    KVB = [0] + [PH_KV + 32 * i for i in range(NT - 1)] + [W // 4]

    def head_of(u):
        return ((u >> 2) & 1) * (H // 2) + (u >> 3)

    def kv_start(u, j):
        row = (u & (B - 1)) * H + head_of(u)
        slot = u & (NSLOT - 1)
        n = KVB[j + 1] - KVB[j]
        src = pl.ds((S - W) // 4 + KVB[j], n)
        dst = pl.ds(KVB[j], n)
        cp(k_hbm.at[row, src], kvbuf.at[NSLOT + slot, dst], S_K + slot).start(priority=0)
        cp(v_hbm.at[row, src], kvbuf.at[slot, dst], S_V + slot).start(priority=1)

    def skew(v, t):
        e = t % G
        return v + L + (G - 1 - e), e * (NT // G) + t // G

    def k_wait(u):
        slot = u & (NSLOT - 1)
        wait_all(kvbuf.at[NSLOT + slot], S_K + slot)

    def v_wait(u):
        slot = u & (NSLOT - 1)
        wait_all(kvbuf.at[slot], S_V + slot)

    def kv_tile(slot, t):
        w = pltpu.bitcast(kvbuf[slot, pl.ds(t * 32, 32)], jnp.uint32)
        return pltpu.bitcast(jnp.concatenate([w[i] for i in range(32)], axis=0), bf16)

    small = [cp(x_hbm, x_v, S_X), cp(c_hbm, c_v, S_C), cp(b1_hbm, b1_v, S_B1), cp(b2_hbm, b2_v, S_B2)]
    HQ = N_WQ // 2
    NM = (N_WM - PH_WM) // PT // 2
    M1 = PH_WM + (NM + 1) * PT
    assert N_WO == N_WQ and HQ % PT == 0 and 0 < N_WM - (M1 + NM * PT) <= PT and NM <= HQ // PT

    def pro2(i):
        wq_p(i * PT, 0)
        wq_p(HQ + i * PT, 1)
        wo_p(i * PT, 0)
        wo_p(HQ + i * PT, 1)

    def pro3(i):
        pro2(i)
        wm_p(PH_WM + i * PT, 0)
        wm_p(M1 + i * PT, 1)

    def pro3_paced(i, z):
        for start, lo0, lo1 in ((wq_p, 0, HQ), (wo_p, 0, HQ), (wm_p, PH_WM, M1)):
            start(lo0 + i * PT, 0)
            start(lo1 + i * PT, 1)
            z = lax.fori_loop(0, SPIN, lambda j, c: (c * 5 + j) & 1023, z)
        return z
    spin_s[0] = lax.fori_loop(0, NPACED, pro3_paced, jnp.int32(1))
    loop(NPACED, NM, pro3)
    for s in small:
        s.start(priority=0)
    wm_p(PH_WM + NM * PT, 0)
    wm_p(M1 + NM * PT, 1, N_WM - (M1 + NM * PT))
    wm_p(0, 0, PH_WM)
    loop(NM, HQ // PT, pro2)

    def kv_prologue(v):
        for t in range(NT):
            u, j = skew(v, t)
            pl.when(u >= 0)(functools.partial(kv_start, u, j))
    V0 = -(L + G - 1)
    VA = min(0, V0 + UA)
    loop(V0, VA, kv_prologue)

    for s in small:
        s.wait()
    wait_all(wm_v, S_WM)
    pad = jnp.zeros((8 - B, D), f32)
    cvec = jnp.concatenate([c_v[...].astype(f32), pad], axis=0)
    x = jnp.concatenate([x_v[...].astype(f32), pad], axis=0)
    mod = _matmul_cols((cvec * jax.nn.sigmoid(cvec)).astype(bf16), _cols(wm_v, 0, D // 8, 6 * CT))
    sa, ca, ga, sb, cb, gb = [mod[:, i * D:(i + 1) * D] for i in range(6)]
    h1 = (_ln(x) * (1.0 + ca) + sa).astype(bf16)
    wait_all(wq_v, S_WQ)
    for h, wc in enumerate(_cols(wq_v, 0, D // 8, H)):
        q_s[h] = jnp.dot(h1, wc, preferred_element_type=f32)
    att_s[...] = jnp.zeros(att_s.shape, f32)
    if VA < 0:
        loop(VA, 0, kv_prologue)

    cexp = (DH ** -0.5) * LOG2E
    row = lax.broadcasted_iota(jnp.int32, (8, DH), 0)

    def qk_tile(qh, u, t):
        return lax.dot_general(qh, kv_tile(NSLOT + (u & (NSLOT - 1)), t), NT_DIMS, preferred_element_type=f32)

    def project(u, acc, lsum):
        l = jnp.sum(lsum, axis=-1, keepdims=True)
        o = jnp.where(row == (u & (B - 1)), acc / l, 0.0).astype(bf16)
        h = head_of(jnp.maximum(u, 0))
        return _matmul_cols(o, _cols(wo_v, h * (DH // 8 * CT), DH // 8, CT))

    def make_body(issue, last=False):
        def body(u, carry):
            mx, acc_p, lsum_p = carry
            par = u & 1
            m = jnp.max(mx, axis=-1, keepdims=True)
            if not last:
                k_wait(u + 1)
                qn = q_s[head_of(u + 1)].astype(bf16)
            v_wait(u)
            att_s[...] += project(u - 1, acc_p, lsum_p)
            mxn = lsum = acc = None
            for t in range(NT):
                if not last:
                    st = qk_tile(qn, u + 1, t)
                    s_s[1 - par, t] = st
                    mxn = st if mxn is None else jnp.maximum(mxn, st)
                p = jnp.exp2((s_s[par, t] - m) * cexp)
                lsum = p if lsum is None else lsum + p
                pv = jnp.dot(p.astype(bf16), kv_tile(u & (NSLOT - 1), t), preferred_element_type=f32)
                acc = pv if acc is None else acc + pv
                issue(u, t)
            return (mx if last else mxn), acc, lsum
        return body

    wait_all(wo_v, S_WO)
    k_wait(0)
    q0 = q_s[0].astype(bf16)
    mx = None
    for t in range(NT):
        st = qk_tile(q0, 0, t)
        s_s[0, t] = st
        mx = st if mx is None else jnp.maximum(mx, st)

    VM = NU - (L + G - 1)
    free = [(v, t) for v in range(VM, NU - 1) for t in range(NT) if skew(v, t)[0] >= NU]
    N1 = (N_W1 - PH_W1) // PT
    N2 = (N_W2 - PH_W2) // PT
    assert SK1 + N1 <= len(free) and SK2 + N2 <= len(free) and N1 >= 64 and N2 >= 3 * NS2
    assert all((i * 43) >> 7 == i // 3 for i in range(N2))

    def slot_index(d, t, minimum, where):
        nfree = minimum(d + 1, G)
        before = where(d < G, d * (d + 1) // 2 * (NT // G), (G * (G - 1) // 2) * (NT // G) + (d - (G - 1)) * NT)
        return before + (t // G) * nfree + (t % G)
    for i, (v, t) in enumerate(free):
        assert slot_index(v - VM, t, min, lambda c, a, b: a if c else b) == i

    W2B = [0] + [PH_W2 + (s * NS2 + o) * PT for s in range(3) for o in (RB2, NS2)] + [N_W2]
    W2G = [0, 1, 0, 1, 0, 1, 2]
    W2R = [[], [], []]
    for r in range(0, F, 128):
        r1 = min(r + 128, F)
        g = max(W2G[i] for i in range(7) if W2B[i] < r1 // 8 * CT and W2B[i + 1] > r // 8 * CT)
        if W2R[g] and W2R[g][-1][1] == r:
            W2R[g][-1][1] = r1
        else:
            W2R[g].append([r, r1])

    def issue_main(v, t):
        kv_start(*skew(v, t))

    def issue_end(v, t):
        u, j = skew(v, t)
        pl.when(u < NU)(functools.partial(kv_start, u, j))
        idx = slot_index(v - VM, t, jnp.minimum, jnp.where)

        @pl.when(jnp.logical_and(u >= NU, jnp.logical_and(idx >= SK1, idx < SK1 + N1)))
        def _():
            i = idx - SK1
            w1_p(PH_W1 + jnp.where(i < 64, (i & 3) * 16 + (i >> 2), i) * PT, 0)

        @pl.when(jnp.logical_and(u >= NU, jnp.logical_and(idx >= SK2, idx < SK2 + N2)))
        def _():
            i = idx - SK2
            rnd = (i * 43) >> 7
            rr = i < 3 * NS2
            st = i - 3 * rnd
            w2_p(PH_W2 + jnp.where(rr, st * NS2 + rnd, i) * PT, 1,
                 g=jnp.where(rr, 2 * st + (rnd >= RB2).astype(jnp.int32), 6))

        @pl.when(jnp.logical_and(u >= NU, idx == SK2 + N2 - 1))
        def _():
            w2_p(PH_W2 + N2 * PT, 1, N_W2 - PH_W2 - N2 * PT, g=6)

    carry = (mx, jnp.zeros((8, DH), f32), jnp.ones((8, DH), f32))
    carry = lax.fori_loop(0, VM, make_body(issue_main), carry)
    w1_p(0, 0, PH_W1)
    w1_p(PH_W1 + N1 * PT, 0, N_W1 - PH_W1 - N1 * PT)
    w2_p(0, 1, PH_W2)
    carry = lax.fori_loop(VM, NU - 1, make_body(issue_end), carry)
    _, acc, lsum = make_body(lambda u, t: None, last=True)(jnp.int32(NU - 1), carry)
    att = att_s[...] + project(jnp.int32(NU - 1), acc, lsum)

    x2 = x + ga * att
    h2 = (_ln(x2) * (1.0 + cb) + sb).astype(bf16)
    wait_all(w1_v, S_W1)
    hh = b1_v[...].astype(f32).reshape(1, F)
    for c, wc in enumerate(_cols(w1_v, 0, F // 8, CT)):
        hh = hh + lax.dot_general(h2[:, c * 128:(c + 1) * 128], wc, NT_DIMS, preferred_element_type=f32)
    hh = jax.nn.gelu(hh, approximate=True).astype(bf16)

    def w2_part(g):
        for i in range(7):
            if W2G[i] == g:
                wait_all(w2_v.at[pl.ds(W2B[i], W2B[i + 1] - W2B[i])], S_W2 + i)
        return sum(_matmul_cols(hh[:, r0:r1], _cols(w2_v, r0 // 8 * CT, (r1 - r0) // 8, CT)) for r0, r1 in W2R[g])
    y = b2_v[...].astype(f32).reshape(1, D) + w2_part(0)
    y = y + w2_part(1)
    out = x2 + gb * y
    out = out + gb * w2_part(2)
    for c in range(CT):
        out_v[:, c * 128:(c + 1) * 128] = out[:, c * 128:(c + 1) * 128].astype(bf16)[0:B]
    co = cp(out_v, o_hbm, S_OUT)
    co.start()
    co.wait()


def _tiles(w):
    r, c = w.shape
    return w.reshape(r // 8, 8, c // 128, 128).transpose(0, 2, 1, 3).reshape(-1, 8, 128)


@jax.jit
def pallas_adaLN_cond__sliding_block_cached__dense_activation_gelu__decode_kernel(A_x, A_k_cache, A_v_cache, A_wq, A_wo, B_x, B_w1, B_b1, B_w2, B_b2, c, w_mod):
    out = pl.pallas_call(
        _kernel,
        in_specs=[pl.BlockSpec(memory_space=pl.ANY)] * 11,
        out_specs=pl.BlockSpec(memory_space=pl.ANY),
        out_shape=jax.ShapeDtypeStruct((B, D), bf16),
        scratch_shapes=[
            pltpu.VMEM((B, D), bf16), pltpu.VMEM((B, D), bf16), pltpu.VMEM((F,), bf16), pltpu.VMEM((D,), bf16),
            pltpu.VMEM((N_WQ, 8, 128), bf16), pltpu.VMEM((N_WO, 8, 128), bf16), pltpu.VMEM((N_W1, 8, 128), bf16),
            pltpu.VMEM((N_W2, 8, 128), bf16), pltpu.VMEM((N_WM, 8, 128), bf16),
            pltpu.VMEM((2 * NSLOT, W // 4, 4, DH), bf16),
            pltpu.VMEM((H, 8, DH), f32), pltpu.VMEM((8, D), f32), pltpu.VMEM((2, NT, 8, 128), f32),
            pltpu.VMEM((B, D), bf16), pltpu.SMEM((1,), jnp.int32),
            pltpu.SemaphoreType.DMA((NSEM,)),
        ],
        compiler_params=pltpu.CompilerParams(vmem_limit_bytes=64 * 1024 * 1024, disable_bounds_checks=True,
                                             disable_semaphore_checks=True),
    )(A_x.reshape(B, D), c, B_b1, B_b2,
      A_k_cache.reshape(B * H, S // 4, 4, DH), A_v_cache.reshape(B * H, S // 4, 4, DH),
      _tiles(A_wq), _tiles(A_wo), _tiles(B_w1.T), _tiles(B_w2), _tiles(w_mod))
    return out.reshape(B, 1, D)
```

```python
import functools

import jax
import jax.numpy as jnp
from jax import lax
import jax.experimental.pallas as pl
import jax.experimental.pallas.tpu as pltpu

B, D, H, S, DH, F = 4, 640, 32, 8192, 128, 1728
W = min(4096, max(256, S // 4))
NT = W // 128
NU = B * H
NSLOT = 16
G = 4
EPS = 1e-5
LOG2E = 1.4426950408889634
bf16 = jnp.bfloat16
f32 = jnp.float32
NT_DIMS = (((1,), (1,)), ((), ()))

PT = 16
CT = D // 128
N_WQ, N_WO, N_WM, N_W1, N_W2 = D * H * DH // 1024, H * DH * D // 1024, D * 6 * D // 1024, F * D // 1024, F * D // 1024

L = 5
UA = 6
NPACED, SPIN = 20, 8
SK1, SK2 = 0, 16
NS2, RB2 = 20, 15
PH_KV, PH_WM, PH_W1, PH_W2 = 31, 7, 13, 3

S_X, S_C, S_B1, S_B2, S_WM, S_WQ, S_WO, S_OUT, S_W1, S_W2, S_K, S_V = 0, 1, 2, 3, 4, 5, 6, 7, 8, 9, 16, 32
NSEM = S_V + NSLOT


def _ln(x):
    m = jnp.mean(x, axis=-1, keepdims=True)
    xc = x - m
    v = jnp.mean(xc * xc, axis=-1, keepdims=True)
    return xc / jnp.sqrt(v + EPS)


def _cols(w_v, lo, nslab, ct):
    blk = w_v[pl.ds(lo, nslab * ct)].reshape(nslab, ct, 8, 128)
    return [blk[:, c].reshape(nslab * 8, 128) for c in range(ct)]


def _matmul_cols(a, cols):
    return jnp.concatenate([jnp.dot(a, wc, preferred_element_type=f32) for wc in cols], axis=1)


def _kernel(x_hbm, c_hbm, b1_hbm, b2_hbm, k_hbm, v_hbm, wq_hbm, wo_hbm, w1_hbm, w2_hbm, wm_hbm,
            o_hbm,
            x_v, c_v, b1_v, b2_v, wq_v, wo_v, w1_v, w2_v, wm_v, kvbuf, q_s, att_s, s_s, out_v, spin_s, sem):
    assert 2 <= L and L + G <= NSLOT

    def cp(src, dst, i):
        return pltpu.make_async_copy(src, dst, sem.at[i])

    def wait_all(buf, i):
        pltpu.make_async_copy(buf, buf, sem.at[i]).wait()

    def loop(lo, hi, f):
        def body(i, c):
            f(i)
            return c
        lax.fori_loop(lo, hi, body, 0)

    def wpiece(hbm, vm, s0):
        def start(lo, prio, n=PT, g=0):
            cp(hbm.at[pl.ds(lo, n)], vm.at[pl.ds(lo, n)], s0 + g).start(priority=prio)
        return start
    wq_p = wpiece(wq_hbm, wq_v, S_WQ)
    wo_p = wpiece(wo_hbm, wo_v, S_WO)
    wm_p = wpiece(wm_hbm, wm_v, S_WM)
    w1_p = wpiece(w1_hbm, w1_v, S_W1)
    w2_p = wpiece(w2_hbm, w2_v, S_W2)

    KVB = [0] + [PH_KV + 32 * i for i in range(NT - 1)] + [W // 4]

    def head_of(u):
        return ((u >> 2) & 1) * (H // 2) + (u >> 3)

    def kv_start(prio, u, j):
        hbm, slot0, sem0 = ((k_hbm, NSLOT, S_K), (v_hbm, 0, S_V))[prio]
        row = (u & (B - 1)) * H + head_of(u)
        slot = u & (NSLOT - 1)
        n = KVB[j + 1] - KVB[j]
        cp(hbm.at[row, pl.ds((S - W) // 4 + KVB[j], n)], kvbuf.at[slot0 + slot, pl.ds(KVB[j], n)],
           sem0 + slot).start(priority=prio)

    def quarter(prio, t):
        return t % G if prio == 0 else G - 1 - t % G

    def skew(prio, v, t):
        e = quarter(prio, t)
        return v + L + (G - 1 - e), e * (NT // G) + t // G

    def k_wait(u):
        slot = u & (NSLOT - 1)
        wait_all(kvbuf.at[NSLOT + slot], S_K + slot)

    def v_wait(u):
        slot = u & (NSLOT - 1)
        wait_all(kvbuf.at[slot], S_V + slot)

    def kv_tile(slot, t):
        w = pltpu.bitcast(kvbuf[slot, pl.ds(t * 32, 32)], jnp.uint32)
        return pltpu.bitcast(jnp.concatenate([w[i] for i in range(32)], axis=0), bf16)

    small = [cp(x_hbm, x_v, S_X), cp(c_hbm, c_v, S_C), cp(b1_hbm, b1_v, S_B1), cp(b2_hbm, b2_v, S_B2)]
    HQ = N_WQ // 2
    NM = (N_WM - PH_WM) // PT // 2
    M1 = PH_WM + (NM + 1) * PT
    assert N_WO == N_WQ and HQ % PT == 0 and 0 < N_WM - (M1 + NM * PT) <= PT and NM <= HQ // PT

    def pro2(i):
        wq_p(i * PT, 0)
        wq_p(HQ + i * PT, 1)
        wo_p(i * PT, 0)
        wo_p(HQ + i * PT, 1)

    def pro3(i):
        pro2(i)
        wm_p(PH_WM + i * PT, 0)
        wm_p(M1 + i * PT, 1)

    def pro3_paced(i, z):
        for start, lo0, lo1 in ((wq_p, 0, HQ), (wo_p, 0, HQ), (wm_p, PH_WM, M1)):
            start(lo0 + i * PT, 0)
            start(lo1 + i * PT, 1)
            z = lax.fori_loop(0, SPIN, lambda j, c: (c * 5 + j) & 1023, z)
        return z
    spin_s[0] = lax.fori_loop(0, NPACED, pro3_paced, jnp.int32(1))
    loop(NPACED, NM, pro3)
    for s in small:
        s.start(priority=0)
    wm_p(PH_WM + NM * PT, 0)
    wm_p(M1 + NM * PT, 1, N_WM - (M1 + NM * PT))
    wm_p(0, 0, PH_WM)
    loop(NM, HQ // PT, pro2)

    def kv_prologue(v):
        for t in range(NT):
            for prio in range(2):
                u, j = skew(prio, v, t)
                pl.when(u >= 0)(functools.partial(kv_start, prio, u, j))
    V0 = -(L + G - 1)
    VA = min(0, V0 + UA)
    loop(V0, VA, kv_prologue)

    for s in small:
        s.wait()
    wait_all(wm_v, S_WM)
    pad = jnp.zeros((8 - B, D), f32)
    cvec = jnp.concatenate([c_v[...].astype(f32), pad], axis=0)
    x = jnp.concatenate([x_v[...].astype(f32), pad], axis=0)
    mod = _matmul_cols((cvec * jax.nn.sigmoid(cvec)).astype(bf16), _cols(wm_v, 0, D // 8, 6 * CT))
    sa, ca, ga, sb, cb, gb = [mod[:, i * D:(i + 1) * D] for i in range(6)]
    h1 = (_ln(x) * (1.0 + ca) + sa).astype(bf16)
    wait_all(wq_v, S_WQ)
    for h, wc in enumerate(_cols(wq_v, 0, D // 8, H)):
        q_s[h] = jnp.dot(h1, wc, preferred_element_type=f32)
    att_s[...] = jnp.zeros(att_s.shape, f32)
    if VA < 0:
        loop(VA, 0, kv_prologue)

    cexp = (DH ** -0.5) * LOG2E
    row = lax.broadcasted_iota(jnp.int32, (8, DH), 0)

    def qk_tile(qh, u, t):
        return lax.dot_general(qh, kv_tile(NSLOT + (u & (NSLOT - 1)), t), NT_DIMS, preferred_element_type=f32)

    def project(u, acc, lsum):
        l = jnp.sum(lsum, axis=-1, keepdims=True)
        o = jnp.where(row == (u & (B - 1)), acc / l, 0.0).astype(bf16)
        h = head_of(jnp.maximum(u, 0))
        return _matmul_cols(o, _cols(wo_v, h * (DH // 8 * CT), DH // 8, CT))

    def make_body(issue, last=False):
        def body(u, carry):
            mx, acc_p, lsum_p = carry
            par = u & 1
            m = jnp.max(mx, axis=-1, keepdims=True)
            if not last:
                k_wait(u + 1)
                qn = q_s[head_of(u + 1)].astype(bf16)
            v_wait(u)
            att_s[...] += project(u - 1, acc_p, lsum_p)
            mxn = lsum = acc = None
            for t in range(NT):
                if not last:
                    st = qk_tile(qn, u + 1, t)
                    s_s[1 - par, t] = st
                    mxn = st if mxn is None else jnp.maximum(mxn, st)
                p = jnp.exp2((s_s[par, t] - m) * cexp)
                lsum = p if lsum is None else lsum + p
                pv = jnp.dot(p.astype(bf16), kv_tile(u & (NSLOT - 1), t), preferred_element_type=f32)
                acc = pv if acc is None else acc + pv
                issue(u, t)
            return (mx if last else mxn), acc, lsum
        return body

    wait_all(wo_v, S_WO)
    k_wait(0)
    q0 = q_s[0].astype(bf16)
    mx = None
    for t in range(NT):
        st = qk_tile(q0, 0, t)
        s_s[0, t] = st
        mx = st if mx is None else jnp.maximum(mx, st)

    VM = NU - (L + G - 1)
    free = [[(v, t) for v in range(VM, NU - 1) for t in range(NT) if skew(prio, v, t)[0] >= NU] for prio in range(2)]
    N1 = (N_W1 - PH_W1) // PT
    N2 = (N_W2 - PH_W2) // PT
    assert SK1 + N1 <= len(free[0]) and SK2 + N2 <= len(free[1]) and N1 >= 64 and N2 >= 3 * NS2
    assert all((i * 43) >> 7 == i // 3 for i in range(N2))

    def free_index(prio, d, t, minimum, where):
        nfree = minimum(d + 1, G)
        before = where(d < G, d * (d + 1) // 2 * (NT // G), (G * (G - 1) // 2) * (NT // G) + (d - (G - 1)) * NT)
        return before + (t // G) * nfree + (t % G if prio == 0 else t % G - (G - nfree))
    for prio in range(2):
        for i, (v, t) in enumerate(free[prio]):
            assert free_index(prio, v - VM, t, min, lambda c, a, b: a if c else b) == i

    W2B = [0] + [PH_W2 + (s * NS2 + o) * PT for s in range(3) for o in (RB2, NS2)] + [N_W2]
    W2G = [0, 1, 0, 1, 0, 1, 2]
    W2R = [[], [], []]
    for r in range(0, F, 128):
        r1 = min(r + 128, F)
        g = max(W2G[i] for i in range(7) if W2B[i] < r1 // 8 * CT and W2B[i + 1] > r // 8 * CT)
        if W2R[g] and W2R[g][-1][1] == r:
            W2R[g][-1][1] = r1
        else:
            W2R[g].append([r, r1])

    def issue_main(v, t):
        for prio in range(2):
            kv_start(prio, *skew(prio, v, t))

    def issue_end(v, t):
        u, j = skew(0, v, t)
        i1 = free_index(0, v - VM, t, jnp.minimum, jnp.where) - SK1
        pl.when(u < NU)(functools.partial(kv_start, 0, u, j))

        @pl.when(jnp.logical_and(u >= NU, jnp.logical_and(i1 >= 0, i1 < N1)))
        def _():
            w1_p(PH_W1 + jnp.where(i1 < 64, (i1 & 3) * 16 + (i1 >> 2), i1) * PT, 0)

        u, j = skew(1, v, t)
        i2 = free_index(1, v - VM, t, jnp.minimum, jnp.where) - SK2
        pl.when(u < NU)(functools.partial(kv_start, 1, u, j))

        @pl.when(jnp.logical_and(u >= NU, jnp.logical_and(i2 >= 0, i2 < N2)))
        def _():
            rnd = (i2 * 43) >> 7
            st = i2 - 3 * rnd
            rr = i2 < 3 * NS2
            w2_p(PH_W2 + jnp.where(rr, st * NS2 + rnd, i2) * PT, 1,
                 g=jnp.where(rr, 2 * st + (rnd >= RB2).astype(jnp.int32), 6))

        @pl.when(jnp.logical_and(u >= NU, i2 == N2 - 1))
        def _():
            w2_p(PH_W2 + N2 * PT, 1, N_W2 - PH_W2 - N2 * PT, g=6)

    carry = (mx, jnp.zeros((8, DH), f32), jnp.ones((8, DH), f32))
    carry = lax.fori_loop(0, VM, make_body(issue_main), carry)
    w1_p(0, 0, PH_W1)
    w1_p(PH_W1 + N1 * PT, 0, N_W1 - PH_W1 - N1 * PT)
    w2_p(0, 1, PH_W2)
    carry = lax.fori_loop(VM, NU - 1, make_body(issue_end), carry)
    _, acc, lsum = make_body(lambda u, t: None, last=True)(jnp.int32(NU - 1), carry)
    att = att_s[...] + project(jnp.int32(NU - 1), acc, lsum)

    x2 = x + ga * att
    h2 = (_ln(x2) * (1.0 + cb) + sb).astype(bf16)
    wait_all(w1_v, S_W1)
    hh = b1_v[...].astype(f32).reshape(1, F)
    for c, wc in enumerate(_cols(w1_v, 0, F // 8, CT)):
        hh = hh + lax.dot_general(h2[:, c * 128:(c + 1) * 128], wc, NT_DIMS, preferred_element_type=f32)
    hh = jax.nn.gelu(hh, approximate=True).astype(bf16)

    def w2_part(g):
        for i in range(7):
            if W2G[i] == g:
                wait_all(w2_v.at[pl.ds(W2B[i], W2B[i + 1] - W2B[i])], S_W2 + i)
        return sum(_matmul_cols(hh[:, r0:r1], _cols(w2_v, r0 // 8 * CT, (r1 - r0) // 8, CT)) for r0, r1 in W2R[g])
    y = b2_v[...].astype(f32).reshape(1, D) + w2_part(0)
    y = y + w2_part(1)
    out = x2 + gb * y
    out = out + gb * w2_part(2)
    for c in range(CT):
        out_v[:, c * 128:(c + 1) * 128] = out[:, c * 128:(c + 1) * 128].astype(bf16)[0:B]
    co = cp(out_v, o_hbm, S_OUT)
    co.start()
    co.wait()


def _tiles(w):
    r, c = w.shape
    return w.reshape(r // 8, 8, c // 128, 128).transpose(0, 2, 1, 3).reshape(-1, 8, 128)


@jax.jit
def pallas_adaLN_cond__sliding_block_cached__dense_activation_gelu__decode_kernel(A_x, A_k_cache, A_v_cache, A_wq, A_wo, B_x, B_w1, B_b1, B_w2, B_b2, c, w_mod):
    out = pl.pallas_call(
        _kernel,
        in_specs=[pl.BlockSpec(memory_space=pl.ANY)] * 11,
        out_specs=pl.BlockSpec(memory_space=pl.ANY),
        out_shape=jax.ShapeDtypeStruct((B, D), bf16),
        scratch_shapes=[
            pltpu.VMEM((B, D), bf16), pltpu.VMEM((B, D), bf16), pltpu.VMEM((F,), bf16), pltpu.VMEM((D,), bf16),
            pltpu.VMEM((N_WQ, 8, 128), bf16), pltpu.VMEM((N_WO, 8, 128), bf16), pltpu.VMEM((N_W1, 8, 128), bf16),
            pltpu.VMEM((N_W2, 8, 128), bf16), pltpu.VMEM((N_WM, 8, 128), bf16),
            pltpu.VMEM((2 * NSLOT, W // 4, 4, DH), bf16),
            pltpu.VMEM((H, 8, DH), f32), pltpu.VMEM((8, D), f32), pltpu.VMEM((2, NT, 8, 128), f32),
            pltpu.VMEM((B, D), bf16), pltpu.SMEM((1,), jnp.int32),
            pltpu.SemaphoreType.DMA((NSEM,)),
        ],
        compiler_params=pltpu.CompilerParams(vmem_limit_bytes=64 * 1024 * 1024, disable_bounds_checks=True,
                                             disable_semaphore_checks=True),
    )(A_x.reshape(B, D), c, B_b1, B_b2,
      A_k_cache.reshape(B * H, S // 4, 4, DH), A_v_cache.reshape(B * H, S // 4, 4, DH),
      _tiles(A_wq), _tiles(A_wo), _tiles(B_w1.T), _tiles(B_w2), _tiles(w_mod))
    return out.reshape(B, 1, D)
```
